```python
import jax
import jax.numpy as jnp

def _softmax(x, axis=-1):
    return jax.nn.softmax(x, axis=axis)
def _gelu(x):
    return jax.nn.gelu(x, approximate=True)
def _silu(x):
    return jax.nn.silu(x)
def _sigmoid(x):
    return jax.nn.sigmoid(x)
def _layernorm(x, axis=-1, eps=1e-5):
    m = jnp.mean(x, axis=axis, keepdims=True)
    v = jnp.var(x, axis=axis, keepdims=True)
    return (x - m) / jnp.sqrt(v + eps)
def _scatter_add(tgt, idx, src, axis=0):
    return tgt.at[idx].add(src)
def _segment_sum(src, seg, n):
    return jax.ops.segment_sum(src, seg, n)
class _Rng:
    def __init__(self, key):
        self._k = key
    def _next(self):
        self._k, sub = jax.random.split(self._k)
        return sub
    def normal(self, shape):
        return jax.random.normal(self._next(), shape, dtype=jnp.bfloat16)
    def randint(self, lo, hi, shape):
        return jax.random.randint(self._next(), shape, lo, hi, dtype=jnp.int32)
    def uniform(self, shape, lo=0.0, hi=1.0):
        return jax.random.uniform(self._next(), shape, jnp.bfloat16, lo, hi)
    def permutation(self, n):
        return jax.random.permutation(self._next(), n)


kernel_name = 'recurrent_scan__ssm_conv_h3__mixer_token_mlp__prompt'

def setup_inputs():
    _rng = _Rng(jax.random.key(int.from_bytes(__import__("os").urandom(4), "little")))
    _w = (lambda a: (lambda t: t.astype(jnp.bfloat16) if jnp.issubdtype(t.dtype, jnp.floating) else t)(jnp.asarray(a)))
    def _A_setup():
        B, S, D = 1, 2048, 576
        ks = 4
        return {
            "q": _w((lambda *s: _rng.normal(s) * 0.05)(B, S, D)),
            "k": _w((lambda *s: _rng.normal(s) * 0.05)(B, S, D)),
            "v": _w((lambda *s: _rng.normal(s) * 0.05)(B, S, D)),
            "shift_k": _w((lambda *s: _rng.normal(s) * 0.05)(D, ks) * 0.5),
            "ssm_k": _w((lambda *s: _rng.normal(s) * 0.05)(D, S) * (1.0 / S ** 0.5)),
            "ssm_D": _w((lambda *s: _rng.normal(s) * 0.05)(D)),
        }
    _A_in = _A_setup()

    def _B_setup():
        B, S, D, F = 1, 2048, 576, 4608
        return {
            "x": _w((lambda *s: _rng.normal(s) * 0.05)(B, S, D)),
            "w1": _w((lambda *s: _rng.normal(s) * 0.05)(S, F) * (S ** -0.5)),
            "b1": _w((lambda *s: _rng.normal(s) * 0.05)(F) * 0.02),
            "w2": _w((lambda *s: _rng.normal(s) * 0.05)(F, S) * (F ** -0.5)),
            "b2": _w((lambda *s: _rng.normal(s) * 0.05)(S) * 0.02),
        }
    _B_in = _B_setup()

    return {
        "A_q": _A_in["q"],
        "A_k": _A_in["k"],
        "A_v": _A_in["v"],
        "A_shift_k": _A_in["shift_k"],
        "A_ssm_k": _A_in["ssm_k"],
        "A_ssm_D": _A_in["ssm_D"],
        "B_x": _B_in["x"],
        "B_w1": _B_in["w1"],
        "B_b1": _B_in["b1"],
        "B_w2": _B_in["w2"],
        "B_b2": _B_in["b2"],
    }

def reference(A_q, A_k, A_v, A_shift_k, A_ssm_k, A_ssm_D, B_x, B_w1, B_b1, B_w2, B_b2):
    def _A_ref(q, k, v, shift_k, ssm_k, ssm_D):
        B, S, D = q.shape
        ks = shift_k.shape[-1]
        k_pad = jnp.pad(k, ((0, 0), (ks - 1, 0), (0, 0)))
        k_shift = jnp.zeros_like(k)
        for t in range(ks):
            k_shift = k_shift + k_pad[:, t:t + S, :] * shift_k[:, ks - 1 - t][None, None, :]
        kv = k_shift * v
        L = 2 * S
        kv_pad = jnp.pad(kv, ((0, 0), (0, S), (0, 0)))
        kf_pad = jnp.pad(ssm_k, ((0, 0), (0, S)))
        kv_f = (lambda x, axes=(-2,-1): jnp.fft.rfft2(x.astype(jnp.float32), axes=axes))(kv_pad[:, None, :, :], axes=(1, 2))
        kf_f = (lambda x, axes=(-2,-1): jnp.fft.rfft2(x.astype(jnp.float32), axes=axes))(kf_pad[:, None, :], axes=(1, 2))
        kf_f = (lambda x, *d: x.transpose(*d))(kf_f, 1, 2, 0)
        y_f = kv_f * kf_f[None, :, :, :]
        y = (lambda x, s, axes=(-2,-1): jnp.fft.irfft2(x, s=s, axes=axes).astype(jnp.bfloat16))(y_f, (1, L), axes=(1, 2))[:, 0, :S, :]
        y = y + kv * ssm_D[None, None, :]
        return q * y

    def _B_ref(x, w1, b1, w2, b2):
        B, S, D = x.shape
        h = _layernorm(x, axis=-1)
        u = jnp.einsum("bsd,sf->bdf", h, w1) + b1
        u = _gelu(u)
        y = jnp.einsum("bdf,fs->bds", u, w2) + b2
        return (lambda x, *d: x.transpose(*d))(y, 0, 2, 1)

    x = A_q
    xn = _layernorm(x, axis=-1)
    s = _A_ref(xn, A_k, A_v, A_shift_k, A_ssm_k, A_ssm_D)
    g = _silu(_B_ref(xn, B_w1, B_b1, B_w2, B_b2))
    return x + s * g
```

```python
import functools

import jax
import jax.numpy as jnp
import numpy as np
from jax import lax
import jax.experimental.pallas as pl
import jax.experimental.pallas.tpu as pltpu

S, D, F, KS = 2048, 576, 4608, 4
C = 128
NB = S // C
FC = 512
N1 = F // FC
RG = D // N1
SC = 256
N2 = S // SC
TC = 256
PR = 16
EPS = 1e-5

f32 = jnp.float32
bf16 = jnp.bfloat16


def _dft_mats():
    t = np.arange(C, dtype=np.float64)
    th = 2.0 * np.pi * (np.arange(C, dtype=np.float64) + 0.5) / (2 * C)
    fw = np.concatenate([np.cos(np.outer(t, th)), -np.sin(np.outer(t, th))], axis=1)
    iv = np.concatenate([np.cos(np.outer(th, t)), -np.sin(np.outer(th, t))], axis=0) / C
    return fw.astype(np.float32), iv.astype(np.float32)


def _gelu(x):
    c = 0.7978845608028654
    return 0.5 * x * (1.0 + jnp.tanh(c * (x + 0.044715 * (x * x * x))))


def _kernel(x_hbm, k_hbm, v_hbm, sk_hbm, w1_hbm, w2_hbm,
            shift_ref, d_ref, b1_ref, b2_ref, fw_ref, iv_ref,
            o_hbm,
            xbuf, kbuf, vbuf, skbuf, w1buf, w2buf, obuf,
            hT, xnT, kvB, ubuf, sT, xf, kf, pk, px, zb, dcol, wsh,
            sem_in, sem_w1, sem_w2, sem_o):
    def w1_copy(c):
        return pltpu.make_async_copy(
            w1_hbm.at[:, pl.ds(pl.multiple_of(c * FC, FC), FC)], w1buf.at[c], sem_w1.at[c])

    def w2_copy(p):
        return pltpu.make_async_copy(
            w2_hbm.at[:, pl.ds(pl.multiple_of(p * SC, SC), SC)], w2buf.at[p], sem_w2.at[p])

    def o_copy(p):
        sl = pl.ds(pl.multiple_of(p * SC, SC), SC)
        return pltpu.make_async_copy(obuf.at[sl, :], o_hbm.at[sl, :], sem_o.at[p])

    x_cp = pltpu.make_async_copy(x_hbm, xbuf, sem_in.at[0])
    k_cp = pltpu.make_async_copy(k_hbm, kbuf.at[pl.ds(16, S), :], sem_in.at[1])
    v_cp = pltpu.make_async_copy(v_hbm, vbuf, sem_in.at[2])
    sk_cp = pltpu.make_async_copy(sk_hbm, skbuf, sem_in.at[3])
    x_cp.start()
    w1_copy(0).start()
    k_cp.start()
    v_cp.start()
    sk_cp.start()
    w1_copy(1).start()

    kbuf[pl.ds(0, 16), :] = jnp.zeros((16, D), bf16)
    dcol[...] = jnp.broadcast_to(d_ref[...].astype(f32), (C, D)).T
    wsh[...] = shift_ref[...].astype(f32).T

    x_cp.wait()

    def ln_body(i, _):
        s0 = pl.multiple_of(i * TC, TC)
        xt = xbuf[pl.ds(s0, TC), :].astype(f32).T
        m = jnp.sum(xt, axis=0, keepdims=True) * (1.0 / D)
        xc = xt - m
        v = jnp.sum(xc * xc, axis=0, keepdims=True) * (1.0 / D)
        r = lax.rsqrt(v + EPS)
        xn = xc * r
        r2 = lax.rsqrt(v * (r * r) + EPS)
        xnT[:, pl.ds(s0, TC)] = xn.astype(bf16)
        hT[:, pl.ds(s0, TC)] = (xn * r2).astype(bf16)
        return 0

    lax.fori_loop(0, S // TC, ln_body, 0)

    k_cp.wait()
    v_cp.wait()

    def kv_body(i, _):
        s0 = pl.multiple_of(i * TC, TC)
        kk = kbuf[pl.ds(s0, TC + 16), :].astype(f32)
        acc = kk[16:, :] * wsh[0:1, :]
        for j in range(1, KS):
            acc = acc + pltpu.roll(kk, j, axis=0)[16:, :] * wsh[j:j + 1, :]
        kv = acc * vbuf[pl.ds(s0, TC), :].astype(f32)
        kvt = kv.T.astype(bf16)
        for b in range(TC // C):
            kvB[i * (TC // C) + b] = kvt[:, b * C:(b + 1) * C]
        return 0

    lax.fori_loop(0, S // TC, kv_body, 0)
    sk_cp.wait()

    sgn = 1.0 - 2.0 * (lax.broadcasted_iota(jnp.int32, (PR, C), 1) & 1).astype(f32)

    def p1_body(c, _):
        @pl.when(c + 2 < N1)
        def _():
            w1_copy(c + 2).start()

        @pl.when(c < N2)
        def _():
            w2_copy(c).start()

        w1_copy(c).wait()
        r0 = pl.multiple_of(c * RG, RG)

        lx = kvB[:, pl.ds(r0, RG), :].reshape(NB * RG, C)
        xf[...] = jnp.dot(lx, fw_ref[...], preferred_element_type=f32)
        lk = jnp.concatenate(
            [skbuf[pl.ds(r0, RG), m * C:(m + 1) * C] for m in range(NB)], axis=0)
        kf[...] = jnp.dot(lk, fw_ref[...], preferred_element_type=f32)

        u = jnp.dot(hT[...], w1buf[c], preferred_element_type=f32)
        u = u + b1_ref[:, pl.ds(pl.multiple_of(c * FC, FC), FC)].astype(f32)
        ubuf[c] = _gelu(u).astype(bf16)

        for pr in range(RG // PR):
            def ld(ref, j, half, pr=pr):
                return ref[j * RG + pr * PR:j * RG + (pr + 1) * PR, half * C:(half + 1) * C]
            dd = dcol[pl.ds(r0 + pr * PR, PR), :]
            kr_prev = ki_prev = None
            for m in range(NB):
                kr = ld(kf, m, 0)
                ki = ld(kf, m, 1)
                if m == 0:
                    kr = kr + dd
                    cc, dm = kr, ki
                else:
                    cc = kr - sgn * ki_prev
                    dm = ki + sgn * kr_prev
                kr_prev, ki_prev = kr, ki
                pk[0, m] = cc
                pk[1, m] = dm - cc
                pk[2, m] = cc + dm
            for j in range(NB):
                px[j] = ld(xf, j, 0) + ld(xf, j, 1)
            for i in range(NB):
                s1 = s2 = s3 = None
                for j in range(i + 1):
                    m = i - j
                    p1 = pk[0, m] * px[j]
                    p2 = ld(xf, j, 0) * pk[1, m]
                    p3 = ld(xf, j, 1) * pk[2, m]
                    if j == 0:
                        s1, s2, s3 = p1, p2, p3
                    else:
                        s1, s2, s3 = s1 + p1, s2 + p2, s3 + p3
                rows = slice(i * RG + pr * PR, i * RG + (pr + 1) * PR)
                zb[rows, 0:C] = (s1 - s3).astype(bf16)
                zb[rows, C:2 * C] = (s1 + s2).astype(bf16)

        y = jnp.dot(zb[...], iv_ref[...], preferred_element_type=f32)
        for i in range(NB):
            q = xnT[pl.ds(r0, RG), i * C:(i + 1) * C].astype(f32)
            sT[pl.ds(r0, RG), i * C:(i + 1) * C] = q * y[i * RG:(i + 1) * RG, :]
        return 0

    lax.fori_loop(0, N1, p1_body, 0)

    def p2_body(p, _):
        w2_copy(p).wait()
        s0 = pl.multiple_of(p * SC, SC)
        acc = jnp.dot(ubuf[0], w2buf[p, 0:FC, :], preferred_element_type=f32)
        for c in range(1, N1):
            acc = acc + jnp.dot(ubuf[c], w2buf[p, c * FC:(c + 1) * FC, :],
                                preferred_element_type=f32)
        y = acc + b2_ref[:, pl.ds(s0, SC)].astype(f32)
        g = y * jax.nn.sigmoid(y)
        pt = (sT[:, pl.ds(s0, SC)] * g).T
        obuf[pl.ds(s0, SC), :] = (xbuf[pl.ds(s0, SC), :].astype(f32) + pt).astype(bf16)
        o_copy(p).start()
        return 0

    lax.fori_loop(0, N2, p2_body, 0)
    for p in range(N2):
        o_copy(p).wait()


def pallas_recurrent_scan__ssm_conv_h3__mixer_token_mlp__prompt_kernel(
    A_q: jax.Array,
    A_k: jax.Array,
    A_v: jax.Array,
    A_shift_k: jax.Array,
    A_ssm_k: jax.Array,
    A_ssm_D: jax.Array,
    B_x: jax.Array,
    B_w1: jax.Array,
    B_b1: jax.Array,
    B_w2: jax.Array,
    B_b2: jax.Array,
):
    del B_x
    fw, iv = _dft_mats()
    any_spec = pl.BlockSpec(memory_space=pl.ANY)
    vmem_spec = pl.BlockSpec(memory_space=pltpu.VMEM)
    out = pl.pallas_call(
        _kernel,
        out_shape=jax.ShapeDtypeStruct((S, D), bf16),
        in_specs=[any_spec] * 6 + [vmem_spec] * 6,
        out_specs=any_spec,
        scratch_shapes=[
            pltpu.VMEM((S, D), bf16),
            pltpu.VMEM((S + 16, D), bf16),
            pltpu.VMEM((S, D), bf16),
            pltpu.VMEM((D, S), bf16),
            pltpu.VMEM((N1, S, FC), bf16),
            pltpu.VMEM((N2, F, SC), bf16),
            pltpu.VMEM((S, D), bf16),
            pltpu.VMEM((D, S), bf16),
            pltpu.VMEM((D, S), bf16),
            pltpu.VMEM((NB, D, C), bf16),
            pltpu.VMEM((N1, D, FC), bf16),
            pltpu.VMEM((D, S), f32),
            pltpu.VMEM((NB * RG, 2 * C), f32),
            pltpu.VMEM((NB * RG, 2 * C), f32),
            pltpu.VMEM((3, NB, PR, C), f32),
            pltpu.VMEM((NB, PR, C), f32),
            pltpu.VMEM((NB * RG, 2 * C), bf16),
            pltpu.VMEM((D, C), f32),
            pltpu.VMEM((KS, D), f32),
            pltpu.SemaphoreType.DMA((4,)),
            pltpu.SemaphoreType.DMA((N1,)),
            pltpu.SemaphoreType.DMA((N2,)),
            pltpu.SemaphoreType.DMA((N2,)),
        ],
        compiler_params=pltpu.CompilerParams(vmem_limit_bytes=110 * 1024 * 1024),
    )(
        A_q.reshape(S, D), A_k.reshape(S, D), A_v.reshape(S, D), A_ssm_k, B_w1, B_w2,
        A_shift_k, A_ssm_D.reshape(1, D), B_b1.reshape(1, F), B_b2.reshape(1, S),
        jnp.asarray(fw, bf16), jnp.asarray(iv, bf16),
    )
    return out.reshape(1, S, D)
```

```python
import functools

import jax
import jax.numpy as jnp
import numpy as np
from jax import lax
import jax.experimental.pallas as pl
import jax.experimental.pallas.tpu as pltpu

S, D, F, KS = 2048, 576, 4608, 4
C = 128
NB = S // C
FC = 512
N1 = F // FC
RG = D // N1
SC = 256
N2 = S // SC
TC = 256
PR = 16
EPS = 1e-5

f32 = jnp.float32
bf16 = jnp.bfloat16


def _dft_mats():
    t = np.arange(C, dtype=np.float64)
    th = 2.0 * np.pi * (np.arange(C, dtype=np.float64) + 0.5) / (2 * C)
    fw = np.concatenate([np.cos(np.outer(t, th)), -np.sin(np.outer(t, th))], axis=1)
    iv = np.concatenate([np.cos(np.outer(th, t)), -np.sin(np.outer(th, t))], axis=0) / C
    return fw.astype(np.float32), iv.astype(np.float32)


def _gelu(x):
    c = 0.7978845608028654
    return 0.5 * x * (1.0 + jnp.tanh(c * (x + 0.044715 * (x * x * x))))


def _kernel(x_hbm, k_hbm, v_hbm, sk_hbm, w1_hbm, w2_hbm,
            shift_ref, d_ref, b1_ref, b2_ref, fw_ref, iv_ref,
            o_hbm,
            xbuf, kbuf, vbuf, skbuf, w1buf, w2buf, obuf,
            hT, xnT, kvB, ubuf, sT, xf, kf, pk, px, zb, dcol, wsh, b1s, b2s,
            sem_in, sem_w1, sem_w2, sem_o):
    def w1_copy(c):
        return pltpu.make_async_copy(
            w1_hbm.at[:, pl.ds(pl.multiple_of(c * FC, FC), FC)], w1buf.at[c], sem_w1.at[c])

    def w2_copy(p):
        return pltpu.make_async_copy(
            w2_hbm.at[:, pl.ds(pl.multiple_of(p * SC, SC), SC)], w2buf.at[p], sem_w2.at[p])

    def o_copy(p):
        sl = pl.ds(pl.multiple_of(p * SC, SC), SC)
        return pltpu.make_async_copy(obuf.at[:, sl], o_hbm.at[:, sl], sem_o.at[p])

    x_cp = pltpu.make_async_copy(x_hbm, xbuf, sem_in.at[0])
    k_cp = pltpu.make_async_copy(k_hbm, kbuf.at[:, pl.ds(C, S)], sem_in.at[1])
    v_cp = pltpu.make_async_copy(v_hbm, vbuf, sem_in.at[2])
    sk_cp = pltpu.make_async_copy(sk_hbm, skbuf, sem_in.at[3])
    x_cp.start()
    w1_copy(0).start()
    k_cp.start()
    v_cp.start()
    sk_cp.start()
    w1_copy(1).start()

    kbuf[:, 0:C] = jnp.zeros((D, C), bf16)
    dcol[...] = jnp.broadcast_to(d_ref[...].astype(f32).reshape(1, D), (C, D)).T
    sh = shift_ref[...].astype(f32)
    for j in range(KS):
        wsh[j] = jnp.broadcast_to(sh[j:j + 1, :], (C, D)).T
    b1s[...] = b1_ref[...].astype(f32)
    b2s[...] = b2_ref[...].astype(f32)

    x_cp.wait()

    def ln_body(i, _):
        s0 = pl.multiple_of(i * TC, TC)
        xt = xbuf[:, pl.ds(s0, TC)].astype(f32)
        m = jnp.sum(xt, axis=0, keepdims=True) * (1.0 / D)
        xc = xt - m
        v = jnp.sum(xc * xc, axis=0, keepdims=True) * (1.0 / D)
        r = lax.rsqrt(v + EPS)
        xn = xc * r
        r2 = lax.rsqrt(v * (r * r) + EPS)
        xnT[:, pl.ds(s0, TC)] = xn.astype(bf16)
        hT[:, pl.ds(s0, TC)] = (xn * r2).astype(bf16)
        return 0

    lax.fori_loop(0, S // TC, ln_body, 0)

    k_cp.wait()
    v_cp.wait()

    def kv_body(i, _):
        s0 = pl.multiple_of(i * TC, TC)
        kk = kbuf[:, pl.ds(s0, TC + C)].astype(f32)
        nt = TC // C
        acc = kk[:, C:] * jnp.concatenate([wsh[0]] * nt, axis=1)
        for j in range(1, KS):
            acc = acc + pltpu.roll(kk, j, axis=1)[:, C:] * jnp.concatenate([wsh[j]] * nt, axis=1)
        kv = (acc * vbuf[:, pl.ds(s0, TC)].astype(f32)).astype(bf16)
        for b in range(nt):
            kvB[i * nt + b] = kv[:, b * C:(b + 1) * C]
        return 0

    lax.fori_loop(0, S // TC, kv_body, 0)
    sk_cp.wait()

    sgn = 1.0 - 2.0 * (lax.broadcasted_iota(jnp.int32, (PR, C), 1) & 1).astype(f32)

    def p1_body(c, _):
        @pl.when(c + 2 < N1)
        def _():
            w1_copy(c + 2).start()

        @pl.when(c < N2)
        def _():
            w2_copy(c).start()

        w1_copy(c).wait()
        r0 = pl.multiple_of(c * RG, RG)

        lx = kvB[:, pl.ds(r0, RG), :].reshape(NB * RG, C)
        xf[...] = jnp.dot(lx, fw_ref[...], preferred_element_type=f32)
        lk = jnp.concatenate(
            [skbuf[pl.ds(r0, RG), m * C:(m + 1) * C] for m in range(NB)], axis=0)
        kf[...] = jnp.dot(lk, fw_ref[...], preferred_element_type=f32)

        u = jnp.dot(hT[...], w1buf[c], preferred_element_type=f32)
        nt = FC // C
        b1c = b1s[pl.ds(c * nt, nt), :]
        u = u + jnp.concatenate([b1c[t:t + 1, :] for t in range(nt)], axis=1)
        ubuf[c] = _gelu(u).astype(bf16)

        for pr in range(RG // PR):
            def ld(ref, j, half, pr=pr):
                return ref[j * RG + pr * PR:j * RG + (pr + 1) * PR, half * C:(half + 1) * C]
            dd = dcol[pl.ds(r0 + pr * PR, PR), :]
            kr_prev = ki_prev = None
            for m in range(NB):
                kr = ld(kf, m, 0)
                ki = ld(kf, m, 1)
                if m == 0:
                    kr = kr + dd
                    cc, dm = kr, ki
                else:
                    cc = kr - sgn * ki_prev
                    dm = ki + sgn * kr_prev
                kr_prev, ki_prev = kr, ki
                pk[0, m] = cc
                pk[1, m] = dm - cc
                pk[2, m] = cc + dm
            for j in range(NB):
                px[j] = ld(xf, j, 0) + ld(xf, j, 1)
            for i in range(NB):
                s1 = s2 = s3 = None
                for j in range(i + 1):
                    m = i - j
                    p1 = pk[0, m] * px[j]
                    p2 = ld(xf, j, 0) * pk[1, m]
                    p3 = ld(xf, j, 1) * pk[2, m]
                    if j == 0:
                        s1, s2, s3 = p1, p2, p3
                    else:
                        s1, s2, s3 = s1 + p1, s2 + p2, s3 + p3
                rows = slice(i * RG + pr * PR, i * RG + (pr + 1) * PR)
                zb[rows, 0:C] = (s1 - s3).astype(bf16)
                zb[rows, C:2 * C] = (s1 + s2).astype(bf16)

        y = jnp.dot(zb[...], iv_ref[...], preferred_element_type=f32)
        for i in range(NB):
            q = xnT[pl.ds(r0, RG), i * C:(i + 1) * C].astype(f32)
            sT[pl.ds(r0, RG), i * C:(i + 1) * C] = q * y[i * RG:(i + 1) * RG, :]
        return 0

    lax.fori_loop(0, N1, p1_body, 0)

    def p2_body(p, _):
        w2_copy(p).wait()
        s0 = pl.multiple_of(p * SC, SC)
        acc = jnp.dot(ubuf[0], w2buf[p, 0:FC, :], preferred_element_type=f32)
        for c in range(1, N1):
            acc = acc + jnp.dot(ubuf[c], w2buf[p, c * FC:(c + 1) * FC, :],
                                preferred_element_type=f32)
        nt = SC // C
        b2c = b2s[pl.ds(p * nt, nt), :]
        y = acc + jnp.concatenate([b2c[t:t + 1, :] for t in range(nt)], axis=1)
        g = y * jax.nn.sigmoid(y)
        pt = sT[:, pl.ds(s0, SC)] * g
        obuf[:, pl.ds(s0, SC)] = (xbuf[:, pl.ds(s0, SC)].astype(f32) + pt).astype(bf16)
        o_copy(p).start()
        return 0

    lax.fori_loop(0, N2, p2_body, 0)
    for p in range(N2):
        o_copy(p).wait()


def pallas_recurrent_scan__ssm_conv_h3__mixer_token_mlp__prompt_kernel(
    A_q: jax.Array,
    A_k: jax.Array,
    A_v: jax.Array,
    A_shift_k: jax.Array,
    A_ssm_k: jax.Array,
    A_ssm_D: jax.Array,
    B_x: jax.Array,
    B_w1: jax.Array,
    B_b1: jax.Array,
    B_w2: jax.Array,
    B_b2: jax.Array,
):
    del B_x
    fw, iv = _dft_mats()
    any_spec = pl.BlockSpec(memory_space=pltpu.HBM)
    vmem_spec = pl.BlockSpec(memory_space=pltpu.VMEM)
    out = pl.pallas_call(
        _kernel,
        out_shape=jax.ShapeDtypeStruct((D, S), bf16),
        in_specs=[any_spec] * 6 + [vmem_spec] * 6,
        out_specs=any_spec,
        scratch_shapes=[
            pltpu.VMEM((D, S), bf16),
            pltpu.VMEM((D, S + C), bf16),
            pltpu.VMEM((D, S), bf16),
            pltpu.VMEM((D, S), bf16),
            pltpu.VMEM((N1, S, FC), bf16),
            pltpu.VMEM((N2, F, SC), bf16),
            pltpu.VMEM((D, S), bf16),
            pltpu.VMEM((D, S), bf16),
            pltpu.VMEM((D, S), bf16),
            pltpu.VMEM((NB, D, C), bf16),
            pltpu.VMEM((N1, D, FC), bf16),
            pltpu.VMEM((D, S), f32),
            pltpu.VMEM((NB * RG, 2 * C), f32),
            pltpu.VMEM((NB * RG, 2 * C), f32),
            pltpu.VMEM((3, NB, PR, C), f32),
            pltpu.VMEM((NB, PR, C), f32),
            pltpu.VMEM((NB * RG, 2 * C), bf16),
            pltpu.VMEM((D, C), f32),
            pltpu.VMEM((KS, D, C), f32),
            pltpu.VMEM((F // C, C), f32),
            pltpu.VMEM((S // C, C), f32),
            pltpu.SemaphoreType.DMA((4,)),
            pltpu.SemaphoreType.DMA((N1,)),
            pltpu.SemaphoreType.DMA((N2,)),
            pltpu.SemaphoreType.DMA((N2,)),
        ],
        compiler_params=pltpu.CompilerParams(vmem_limit_bytes=110 * 1024 * 1024),
    )(
        A_q.reshape(S, D).T, A_k.reshape(S, D).T, A_v.reshape(S, D).T, A_ssm_k, B_w1, B_w2,
        A_shift_k.T, A_ssm_D, B_b1.reshape(F // C, C), B_b2.reshape(S // C, C),
        jnp.asarray(fw, bf16), jnp.asarray(iv, bf16),
    )
    return out.T.reshape(1, S, D)
```

```python
import functools

import jax
import jax.numpy as jnp
import numpy as np
from jax import lax
import jax.experimental.pallas as pl
import jax.experimental.pallas.tpu as pltpu

S, D, F, KS = 2048, 576, 4608, 4
C = 128
NB = S // C
FC = 512
N1 = F // FC
RG = D // N1
SC = 256
N2 = S // SC
TC = 256
PR = 8
EPS = 1e-5
IB = 2

f32 = jnp.float32
bf16 = jnp.bfloat16


def _dft_mats():
    t = np.arange(C, dtype=np.float64)
    th = 2.0 * np.pi * (np.arange(C, dtype=np.float64) + 0.5) / (2 * C)
    fw = np.concatenate([np.cos(np.outer(t, th)), -np.sin(np.outer(t, th))], axis=1)
    iv = np.concatenate([np.cos(np.outer(th, t)), -np.sin(np.outer(th, t))], axis=0) / C
    return fw.astype(np.float32), iv.astype(np.float32)


def _gelu(x):
    c = 0.7978845608028654
    return 0.5 * x * (1.0 + jnp.tanh(c * (x + 0.044715 * (x * x * x))))


def _kernel(x_hbm, k_hbm, v_hbm, sk_hbm, w1_hbm, w2_hbm,
            shift_ref, d_ref, b1_ref, b2_ref, fw_ref, iv_ref,
            o_hbm,
            xbuf, kbuf, vbuf, skbuf, w1buf, w2buf, obuf,
            hT, xnT, kvB, ubuf, sT, xf, kf, pk, px, zb, dcol, wsh, b1s, b2s,
            sem_in, sem_w1, sem_w2, sem_o):
    def w1_copy(c):
        return pltpu.make_async_copy(
            w1_hbm.at[:, pl.ds(pl.multiple_of(c * FC, FC), FC)], w1buf.at[c], sem_w1.at[c])

    def w2_copy(p):
        return pltpu.make_async_copy(
            w2_hbm.at[:, pl.ds(pl.multiple_of(p * SC, SC), SC)], w2buf.at[p], sem_w2.at[p])

    def o_copy(p):
        sl = pl.ds(pl.multiple_of(p * SC, SC), SC)
        return pltpu.make_async_copy(obuf.at[:, sl], o_hbm.at[:, sl], sem_o.at[p])

    x_cp = pltpu.make_async_copy(x_hbm, xbuf, sem_in.at[0])
    k_cp = pltpu.make_async_copy(k_hbm, kbuf.at[:, pl.ds(C, S)], sem_in.at[1])
    v_cp = pltpu.make_async_copy(v_hbm, vbuf, sem_in.at[2])
    sk_cp = pltpu.make_async_copy(sk_hbm, skbuf, sem_in.at[3])
    x_cp.start()
    w1_copy(0).start()
    k_cp.start()
    v_cp.start()
    sk_cp.start()
    w1_copy(1).start()

    kbuf[:, 0:C] = jnp.zeros((D, C), bf16)
    dcol[...] = jnp.broadcast_to(d_ref[...].astype(f32).reshape(1, D), (C, D)).T
    sh = shift_ref[...].astype(f32)
    for j in range(KS):
        wsh[j] = jnp.broadcast_to(sh[j:j + 1, :], (C, D)).T
    b1s[...] = b1_ref[...].astype(f32)
    b2s[...] = b2_ref[...].astype(f32)

    x_cp.wait()

    def ln_body(i, _):
        s0 = pl.multiple_of(i * TC, TC)
        xt = xbuf[:, pl.ds(s0, TC)].astype(f32)
        m = jnp.sum(xt, axis=0, keepdims=True) * (1.0 / D)
        xc = xt - m
        v = jnp.sum(xc * xc, axis=0, keepdims=True) * (1.0 / D)
        r = lax.rsqrt(v + EPS)
        xn = xc * r
        r2 = lax.rsqrt(v * (r * r) + EPS)
        xnT[:, pl.ds(s0, TC)] = xn.astype(bf16)
        hT[:, pl.ds(s0, TC)] = (xn * r2).astype(bf16)
        return 0

    lax.fori_loop(0, S // TC, ln_body, 0)

    k_cp.wait()
    v_cp.wait()

    def kv_body(i, _):
        s0 = pl.multiple_of(i * TC, TC)
        kk = kbuf[:, pl.ds(s0, TC + C)].astype(f32)
        nt = TC // C
        acc = kk[:, C:] * jnp.concatenate([wsh[0]] * nt, axis=1)
        for j in range(1, KS):
            acc = acc + pltpu.roll(kk, j, axis=1)[:, C:] * jnp.concatenate([wsh[j]] * nt, axis=1)
        kv = (acc * vbuf[:, pl.ds(s0, TC)].astype(f32)).astype(bf16)
        for b in range(nt):
            kvB[i * nt + b] = kv[:, b * C:(b + 1) * C]
        return 0

    lax.fori_loop(0, S // TC, kv_body, 0)
    sk_cp.wait()

    sgn = 1.0 - 2.0 * (lax.broadcasted_iota(jnp.int32, (PR, C), 1) & 1).astype(f32)

    def dft(g):
        r0 = pl.multiple_of(g * RG, RG)
        sl = 0
        lx = kvB[:, pl.ds(r0, RG), :].reshape(NB * RG, C)
        xf[sl] = jnp.dot(lx, fw_ref[...], preferred_element_type=f32)
        lk = jnp.concatenate(
            [skbuf[pl.ds(r0, RG), m * C:(m + 1) * C] for m in range(NB)], axis=0)
        kf[sl] = jnp.dot(lk, fw_ref[...], preferred_element_type=f32)

    def idft(g):
        r0 = pl.multiple_of(g * RG, RG)
        y = jnp.dot(zb[0], iv_ref[...], preferred_element_type=f32)
        for i in range(NB):
            q = xnT[pl.ds(r0, RG), i * C:(i + 1) * C].astype(f32)
            sT[pl.ds(r0, RG), i * C:(i + 1) * C] = q * y[i * RG:(i + 1) * RG, :]

    def mac(g, pr, link):
        sl = 0
        r0 = pl.multiple_of(g * RG, RG)
        def ld(ref, j, half):
            return ref[sl, j * RG + pr * PR:j * RG + (pr + 1) * PR, half * C:(half + 1) * C]
        dd = dcol[pl.ds(r0 + pr * PR, PR), :]
        kr_prev = ki_prev = None
        for m in range(NB):
            kr = ld(kf, m, 0)
            ki = ld(kf, m, 1)
            if m == 0:
                kr = kr + dd
                cc, dm = kr, ki
            else:
                cc = kr - sgn * ki_prev
                dm = ki + sgn * kr_prev
            kr_prev, ki_prev = kr, ki
            pk[0, 0, m] = cc
            pk[0, 1, m] = dm - cc
            pk[0, 2, m] = cc + dm
        for j in range(NB):
            px[0, j] = ld(xf, j, 0) + ld(xf, j, 1)
        for i0 in range(0, NB, IB):
            acc = [[None] * 3 for _ in range(IB)]
            kc = {}
            for j in range(i0 + IB):
                a, b_, ab = ld(xf, j, 0), ld(xf, j, 1), px[0, j]
                for t in range(IB):
                    m = i0 + t - j
                    if m < 0:
                        continue
                    if m not in kc:
                        kc[m] = (pk[0, 0, m], pk[0, 1, m], pk[0, 2, m])
                    k0, k1, k2 = kc[m]
                    ps = (k0 * ab, a * k1, b_ * k2)
                    for q in range(3):
                        if acc[t][q] is None:
                            acc[t][q] = ps[q] if link[0] is None else ps[q] + 0.0 * link[0][t][q]
                        else:
                            acc[t][q] = acc[t][q] + ps[q]
                kc = {m: v for m, v in kc.items() if m >= i0 - j}
            link[0] = acc
            for t in range(IB):
                i = i0 + t
                s1, s2, s3 = acc[t]
                rows = slice(i * RG + pr * PR, i * RG + (pr + 1) * PR)
                zb[sl, rows, 0:C] = (s1 - s3).astype(bf16)
                zb[sl, rows, C:2 * C] = (s1 + s2).astype(bf16)

    dft(0)
    zb[...] = jnp.zeros(zb.shape, bf16)

    def p1_body(c, _):
        @pl.when(c + 2 < N1)
        def _():
            w1_copy(c + 2).start()

        @pl.when(c < N2)
        def _():
            w2_copy(c).start()

        w1_copy(c).wait()
        idft(jnp.maximum(c - 1, 0))
        link = [None]
        for pr in range(RG // PR):
            mac(c, pr, link)
        dft(jnp.minimum(c + 1, N1 - 1))
        u = jnp.dot(hT[...], w1buf[c], preferred_element_type=f32)
        nt = FC // C
        b1c = b1s[pl.ds(c * nt, nt), :]
        u = u + jnp.concatenate([b1c[t:t + 1, :] for t in range(nt)], axis=1)
        ubuf[c] = _gelu(u).astype(bf16)
        return 0

    lax.fori_loop(0, N1, p1_body, 0)
    idft(N1 - 1)

    def p2_body(p, _):
        w2_copy(p).wait()
        s0 = pl.multiple_of(p * SC, SC)
        acc = jnp.dot(ubuf[0], w2buf[p, 0:FC, :], preferred_element_type=f32)
        for c in range(1, N1):
            acc = acc + jnp.dot(ubuf[c], w2buf[p, c * FC:(c + 1) * FC, :],
                                preferred_element_type=f32)
        nt = SC // C
        b2c = b2s[pl.ds(p * nt, nt), :]
        y = acc + jnp.concatenate([b2c[t:t + 1, :] for t in range(nt)], axis=1)
        g = y * jax.nn.sigmoid(y)
        pt = sT[:, pl.ds(s0, SC)] * g
        obuf[:, pl.ds(s0, SC)] = (xbuf[:, pl.ds(s0, SC)].astype(f32) + pt).astype(bf16)
        o_copy(p).start()
        return 0

    lax.fori_loop(0, N2, p2_body, 0)
    for p in range(N2):
        o_copy(p).wait()


def pallas_recurrent_scan__ssm_conv_h3__mixer_token_mlp__prompt_kernel(
    A_q: jax.Array,
    A_k: jax.Array,
    A_v: jax.Array,
    A_shift_k: jax.Array,
    A_ssm_k: jax.Array,
    A_ssm_D: jax.Array,
    B_x: jax.Array,
    B_w1: jax.Array,
    B_b1: jax.Array,
    B_w2: jax.Array,
    B_b2: jax.Array,
):
    del B_x
    fw, iv = _dft_mats()
    any_spec = pl.BlockSpec(memory_space=pltpu.HBM)
    vmem_spec = pl.BlockSpec(memory_space=pltpu.VMEM)
    out = pl.pallas_call(
        _kernel,
        out_shape=jax.ShapeDtypeStruct((D, S), bf16),
        in_specs=[any_spec] * 6 + [vmem_spec] * 6,
        out_specs=any_spec,
        scratch_shapes=[
            pltpu.VMEM((D, S), bf16),
            pltpu.VMEM((D, S + C), bf16),
            pltpu.VMEM((D, S), bf16),
            pltpu.VMEM((D, S), bf16),
            pltpu.VMEM((N1, S, FC), bf16),
            pltpu.VMEM((N2, F, SC), bf16),
            pltpu.VMEM((D, S), bf16),
            pltpu.VMEM((D, S), bf16),
            pltpu.VMEM((D, S), bf16),
            pltpu.VMEM((NB, D, C), bf16),
            pltpu.VMEM((N1, D, FC), bf16),
            pltpu.VMEM((D, S), f32),
            pltpu.VMEM((1, NB * RG, 2 * C), f32),
            pltpu.VMEM((1, NB * RG, 2 * C), f32),
            pltpu.VMEM((RG // PR, 3, NB, PR, C), f32),
            pltpu.VMEM((RG // PR, NB, PR, C), f32),
            pltpu.VMEM((1, NB * RG, 2 * C), bf16),
            pltpu.VMEM((D, C), f32),
            pltpu.VMEM((KS, D, C), f32),
            pltpu.VMEM((F // C, C), f32),
            pltpu.VMEM((S // C, C), f32),
            pltpu.SemaphoreType.DMA((4,)),
            pltpu.SemaphoreType.DMA((N1,)),
            pltpu.SemaphoreType.DMA((N2,)),
            pltpu.SemaphoreType.DMA((N2,)),
        ],
        compiler_params=pltpu.CompilerParams(vmem_limit_bytes=110 * 1024 * 1024),
    )(
        A_q.reshape(S, D).T, A_k.reshape(S, D).T, A_v.reshape(S, D).T, A_ssm_k, B_w1, B_w2,
        A_shift_k.T, A_ssm_D, B_b1.reshape(F // C, C), B_b2.reshape(S // C, C),
        jnp.asarray(fw, bf16), jnp.asarray(iv, bf16),
    )
    return out.T.reshape(1, S, D)
```

```python
import jax
import jax.numpy as jnp
import numpy as np
from jax import lax
import jax.experimental.pallas as pl
import jax.experimental.pallas.tpu as pltpu

S, D, F, KS = 2048, 576, 4608, 4
C = 128
NB = S // C
FC = 512
N1 = F // FC
RG = D // N1
SC = 256
N2 = S // SC
TC = 256
NX = S // TC
PR = 8
IB = 2
EPS = 1e-5

f32 = jnp.float32
bf16 = jnp.bfloat16


def _dft_mats():
    t = np.arange(C, dtype=np.float64)
    th = 2.0 * np.pi * (np.arange(C, dtype=np.float64) + 0.5) / (2 * C)
    fw = np.concatenate([np.cos(np.outer(t, th)), -np.sin(np.outer(t, th))], axis=1)
    iv = np.concatenate([np.cos(np.outer(th, t)), -np.sin(np.outer(th, t))], axis=0) / C
    return fw.astype(np.float32), iv.astype(np.float32)


def _gelu(x):
    c = 0.7978845608028654
    return 0.5 * x * (1.0 + jnp.tanh(c * (x + 0.044715 * (x * x * x))))


def _kernel(x_hbm, k_hbm, v_hbm, sk_hbm, w1_hbm, w2_hbm,
            shift_ref, d_ref, b1_ref, b2_ref, fw_ref, iv_ref,
            o_hbm,
            xbuf, kbuf, vbuf, skbuf, w1buf, w2buf, obuf,
            hT, xnT, kvs, ubuf, sT, xf, kf, pk, px, zb, dcol, wsh, b1s, b2s,
            sem_x, sem_g, sem_w1, sem_w2, sem_o):
    def al(i, n):
        return pl.ds(i * n if isinstance(i, int) else pl.multiple_of(i * n, n), n)

    def x_copy(i):
        return pltpu.make_async_copy(x_hbm.at[:, al(i, TC)], xbuf.at[:, al(i, TC)], sem_x.at[i])

    def g_copies(g):
        return [pltpu.make_async_copy(src.at[al(g, RG), :], dst.at[al(g, RG), :], sem_g.at[n, g])
                for n, (src, dst) in enumerate(((k_hbm, kbuf), (v_hbm, vbuf), (sk_hbm, skbuf)))]

    def w1_copy(c):
        return pltpu.make_async_copy(w1_hbm.at[:, al(c, FC)], w1buf.at[c], sem_w1.at[c])

    def w2_copy(p):
        return pltpu.make_async_copy(w2_hbm.at[:, al(p, SC)], w2buf.at[p], sem_w2.at[p])

    def o_copy(p):
        return pltpu.make_async_copy(obuf.at[:, al(p, SC)], o_hbm.at[:, al(p, SC)], sem_o.at[p])

    for i in range(NX):
        x_copy(i).start()
    for cp in g_copies(0):
        cp.start()
    w1_copy(0).start()
    for cp in g_copies(1):
        cp.start()
    w1_copy(1).start()

    dcol[...] = jnp.broadcast_to(d_ref[...].astype(f32).reshape(1, D), (C, D)).T
    sh = shift_ref[...].astype(f32)
    for j in range(KS):
        wsh[j] = jnp.broadcast_to(sh[j:j + 1, :], (C, D)).T
    b1s[...] = b1_ref[...].astype(f32)
    b2s[...] = b2_ref[...].astype(f32)
    zb[...] = jnp.zeros(zb.shape, bf16)

    def ln_body(i, _):
        x_copy(i).wait()
        xt = xbuf[:, al(i, TC)].astype(f32)
        m = jnp.sum(xt, axis=0, keepdims=True) * (1.0 / D)
        xc = xt - m
        v = jnp.sum(xc * xc, axis=0, keepdims=True) * (1.0 / D)
        r = lax.rsqrt(v + EPS)
        xn = xc * r
        r2 = lax.rsqrt(v * (r * r) + EPS)
        xnT[:, al(i, TC)] = xn.astype(bf16)
        hT[:, al(i, TC)] = (xn * r2).astype(bf16)
        return 0

    lax.fori_loop(0, NX, ln_body, 0)

    lane = lax.broadcasted_iota(jnp.int32, (16, C), 1)
    sgn = 1.0 - 2.0 * (lax.broadcasted_iota(jnp.int32, (PR, C), 1) & 1).astype(f32)

    def kv_stage(g):
        r0 = g * RG if isinstance(g, int) else pl.multiple_of(g * RG, RG)
        for sb in range(RG // 16):
            rows = pl.ds(r0 + sb * 16, 16)
            w = [wsh[j, rows, :] for j in range(KS)]
            prev = None
            for t in range(NB):
                kc = kbuf[rows, t * C:(t + 1) * C].astype(f32)
                rolled = [pltpu.roll(kc, j, axis=1) for j in range(1, KS)]
                acc = kc * w[0]
                for j in range(1, KS):
                    if prev is None:
                        shifted = jnp.where(lane < j, 0.0, rolled[j - 1])
                    else:
                        shifted = jnp.where(lane < j, prev[j - 1], rolled[j - 1])
                    acc = acc + shifted * w[j]
                prev = rolled
                kv = acc * vbuf[rows, t * C:(t + 1) * C].astype(f32)
                kvs[t * RG + sb * 16:t * RG + (sb + 1) * 16, :] = kv.astype(bf16)

    def dft_stage(g):
        r0 = g * RG if isinstance(g, int) else pl.multiple_of(g * RG, RG)
        xf[...] = jnp.dot(kvs[...], fw_ref[...], preferred_element_type=f32)
        lk = jnp.concatenate(
            [skbuf[pl.ds(r0, RG), m * C:(m + 1) * C] for m in range(NB)], axis=0)
        kf[...] = jnp.dot(lk, fw_ref[...], preferred_element_type=f32)

    def idft_stage(g):
        r0 = g * RG if isinstance(g, int) else pl.multiple_of(g * RG, RG)
        y = jnp.dot(zb[...], iv_ref[...], preferred_element_type=f32)
        for i in range(NB):
            q = xnT[pl.ds(r0, RG), i * C:(i + 1) * C].astype(f32)
            sT[pl.ds(r0, RG), i * C:(i + 1) * C] = q * y[i * RG:(i + 1) * RG, :]

    def mac_stage(g):
        r0 = g * RG if isinstance(g, int) else pl.multiple_of(g * RG, RG)
        link = None
        for pr in range(RG // PR):
            def ld(ref, j, half, pr=pr):
                return ref[j * RG + pr * PR:j * RG + (pr + 1) * PR, half * C:(half + 1) * C]
            dd = dcol[pl.ds(r0 + pr * PR, PR), :]
            kr_prev = ki_prev = None
            for m in range(NB):
                kr, ki = ld(kf, m, 0), ld(kf, m, 1)
                if m == 0:
                    kr = kr + dd
                    cc, dm = kr, ki
                else:
                    cc = kr - sgn * ki_prev
                    dm = ki + sgn * kr_prev
                kr_prev, ki_prev = kr, ki
                pk[0, m] = cc
                pk[1, m] = dm - cc
                pk[2, m] = cc + dm
            for j in range(NB):
                px[j] = ld(xf, j, 0) + ld(xf, j, 1)
            for i0 in range(0, NB, IB):
                acc = [[None] * 3 for _ in range(IB)]
                kc = {}
                for j in range(i0 + IB):
                    a, b_, ab = ld(xf, j, 0), ld(xf, j, 1), px[j]
                    for t in range(IB):
                        m = i0 + t - j
                        if m < 0:
                            continue
                        if m not in kc:
                            kc[m] = (pk[0, m], pk[1, m], pk[2, m])
                        k0, k1, k2 = kc[m]
                        ps = (k0 * ab, a * k1, b_ * k2)
                        for q in range(3):
                            if acc[t][q] is not None:
                                acc[t][q] = acc[t][q] + ps[q]
                            elif link is None:
                                acc[t][q] = ps[q]
                            else:
                                acc[t][q] = ps[q] + 0.0 * link[t][q]
                    kc = {m: val for m, val in kc.items() if m >= i0 - j}
                link = acc
                for t in range(IB):
                    s1, s2, s3 = acc[t]
                    rows = slice((i0 + t) * RG + pr * PR, (i0 + t) * RG + (pr + 1) * PR)
                    zb[rows, 0:C] = (s1 - s3).astype(bf16)
                    zb[rows, C:2 * C] = (s1 + s2).astype(bf16)

    for cp in g_copies(0):
        cp.wait()
    kv_stage(0)
    dft_stage(0)

    def p1_body(c, _):
        @pl.when(c + 2 < N1)
        def _():
            for cp in g_copies(c + 2):
                cp.start()
            w1_copy(c + 2).start()

        @pl.when(c + 2 >= N1)
        def _():
            w2_copy(c + 2 - N1).start()

        @pl.when(c + 1 < N1)
        def _():
            for cp in g_copies(c + 1):
                cp.wait()

        w1_copy(c).wait()
        idft_stage(jnp.maximum(c - 1, 0))
        mac_stage(c)
        gn = jnp.minimum(c + 1, N1 - 1)
        kv_stage(gn)
        dft_stage(gn)
        u = jnp.dot(hT[...], w1buf[c], preferred_element_type=f32)
        nt = FC // C
        b1c = b1s[pl.ds(c * nt, nt), :]
        u = u + jnp.concatenate([b1c[t:t + 1, :] for t in range(nt)], axis=1)
        ubuf[c] = _gelu(u).astype(bf16)
        return 0

    lax.fori_loop(0, N1, p1_body, 0)
    idft_stage(N1 - 1)

    def p2_body(p, _):
        @pl.when(p + 2 < N2)
        def _():
            w2_copy(p + 2).start()

        w2_copy(p).wait()
        acc = jnp.dot(ubuf[0], w2buf[p, 0:FC, :], preferred_element_type=f32)
        for c in range(1, N1):
            acc = acc + jnp.dot(ubuf[c], w2buf[p, c * FC:(c + 1) * FC, :],
                                preferred_element_type=f32)
        nt = SC // C
        b2c = b2s[pl.ds(p * nt, nt), :]
        y = acc + jnp.concatenate([b2c[t:t + 1, :] for t in range(nt)], axis=1)
        g = y * jax.nn.sigmoid(y)
        obuf[:, al(p, SC)] = (xbuf[:, al(p, SC)].astype(f32) + sT[:, al(p, SC)] * g).astype(bf16)
        o_copy(p).start()
        return 0

    lax.fori_loop(0, N2, p2_body, 0)
    for p in range(N2):
        o_copy(p).wait()


def pallas_recurrent_scan__ssm_conv_h3__mixer_token_mlp__prompt_kernel(
    A_q: jax.Array,
    A_k: jax.Array,
    A_v: jax.Array,
    A_shift_k: jax.Array,
    A_ssm_k: jax.Array,
    A_ssm_D: jax.Array,
    B_x: jax.Array,
    B_w1: jax.Array,
    B_b1: jax.Array,
    B_w2: jax.Array,
    B_b2: jax.Array,
):
    del B_x
    fw, iv = _dft_mats()
    hbm_spec = pl.BlockSpec(memory_space=pltpu.HBM)
    vmem_spec = pl.BlockSpec(memory_space=pltpu.VMEM)
    out = pl.pallas_call(
        _kernel,
        out_shape=jax.ShapeDtypeStruct((D, S), bf16),
        in_specs=[hbm_spec] * 6 + [vmem_spec] * 6,
        out_specs=hbm_spec,
        scratch_shapes=[
            pltpu.VMEM((D, S), bf16),
            pltpu.VMEM((D, S), bf16),
            pltpu.VMEM((D, S), bf16),
            pltpu.VMEM((D, S), bf16),
            pltpu.VMEM((N1, S, FC), bf16),
            pltpu.VMEM((N2, F, SC), bf16),
            pltpu.VMEM((D, S), bf16),
            pltpu.VMEM((D, S), bf16),
            pltpu.VMEM((D, S), bf16),
            pltpu.VMEM((NB * RG, C), bf16),
            pltpu.VMEM((N1, D, FC), bf16),
            pltpu.VMEM((D, S), f32),
            pltpu.VMEM((NB * RG, 2 * C), f32),
            pltpu.VMEM((NB * RG, 2 * C), f32),
            pltpu.VMEM((3, NB, PR, C), f32),
            pltpu.VMEM((NB, PR, C), f32),
            pltpu.VMEM((NB * RG, 2 * C), bf16),
            pltpu.VMEM((D, C), f32),
            pltpu.VMEM((KS, D, C), f32),
            pltpu.VMEM((F // C, C), f32),
            pltpu.VMEM((S // C, C), f32),
            pltpu.SemaphoreType.DMA((NX,)),
            pltpu.SemaphoreType.DMA((3, N1)),
            pltpu.SemaphoreType.DMA((N1,)),
            pltpu.SemaphoreType.DMA((N2,)),
            pltpu.SemaphoreType.DMA((N2,)),
        ],
        compiler_params=pltpu.CompilerParams(vmem_limit_bytes=110 * 1024 * 1024),
    )(
        A_q.reshape(S, D).T, A_k.reshape(S, D).T, A_v.reshape(S, D).T, A_ssm_k, B_w1, B_w2,
        A_shift_k.T, A_ssm_D, B_b1.reshape(F // C, C), B_b2.reshape(S // C, C),
        jnp.asarray(fw, bf16), jnp.asarray(iv, bf16),
    )
    return out.T.reshape(1, S, D)
```

```python
import jax
import jax.numpy as jnp
import numpy as np
from jax import lax
import jax.experimental.pallas as pl
import jax.experimental.pallas.tpu as pltpu

S, D, F, KS = 2048, 576, 4608, 4
C = 128
NB = S // C
FC = 512
N1 = F // FC
RG = D // N1
SC = 256
N2 = S // SC
TC = 256
NX = S // TC
PR = 8
IB = 2
EPS = 1e-5

f32 = jnp.float32
bf16 = jnp.bfloat16


def _dft_mats():
    t = np.arange(C, dtype=np.float64)
    th = 2.0 * np.pi * (np.arange(C, dtype=np.float64) + 0.5) / (2 * C)
    fw = np.concatenate([np.cos(np.outer(t, th)), -np.sin(np.outer(t, th))], axis=1)
    iv = np.concatenate([np.cos(np.outer(th, t)), -np.sin(np.outer(th, t))], axis=0) / C
    return fw.astype(np.float32), iv.astype(np.float32)


def _gelu(x):
    c = 0.7978845608028654
    hx = 0.5 * x
    return hx + hx * jnp.tanh(x * (c + (c * 0.044715) * (x * x)))


def _kernel(x_hbm, k_hbm, v_hbm, sk_hbm, w1_hbm, w2_hbm,
            shift_ref, d_ref, b1_ref, b2_ref, fw_ref, iv_ref,
            o_hbm,
            xbuf, kbuf, vbuf, skbuf, w1buf, w2buf, obuf,
            hT, xnT, kvs, ubuf, sT, xf, kf, pk, px, zb, dcol, wsh, b1s, b2s, zmask,
            sem_x, sem_g, sem_w1, sem_w2, sem_o):
    def al(i, n):
        return pl.ds(i * n if isinstance(i, int) else pl.multiple_of(i * n, n), n)

    def x_copy(i):
        return pltpu.make_async_copy(x_hbm.at[:, al(i, TC)], xbuf.at[:, al(i, TC)], sem_x.at[i])

    def g_copies(g):
        return [pltpu.make_async_copy(src.at[al(g, RG), :], dst.at[al(g, RG), :], sem_g.at[n, g])
                for n, (src, dst) in enumerate(((k_hbm, kbuf), (v_hbm, vbuf), (sk_hbm, skbuf)))]

    def w1_copy(c):
        return pltpu.make_async_copy(w1_hbm.at[:, al(c, FC)], w1buf.at[c], sem_w1.at[c])

    def w2_copy(p):
        return pltpu.make_async_copy(w2_hbm.at[:, al(p, SC)], w2buf.at[p], sem_w2.at[p])

    def o_copy(p):
        return pltpu.make_async_copy(obuf.at[:, al(p, SC)], o_hbm.at[:, al(p, SC)], sem_o.at[p])

    for i in range(NX):
        x_copy(i).start()
    for cp in g_copies(0):
        cp.start()
    w1_copy(0).start()

    dcol[...] = jnp.broadcast_to(d_ref[...].astype(f32).reshape(1, D), (C, D)).T
    sh = shift_ref[...].astype(f32)
    for j in range(KS):
        wsh[j] = jnp.broadcast_to(sh[j:j + 1, :], (C, D)).T
    b1s[...] = b1_ref[...].astype(f32)
    b2s[...] = b2_ref[...].astype(f32)
    zb[...] = jnp.zeros(zb.shape, bf16)
    zmask[...] = jnp.zeros(zmask.shape, jnp.int32)

    def ln_body(i, _):
        x_copy(i).wait()
        xt = xbuf[:, al(i, TC)].astype(f32)
        m = jnp.sum(xt, axis=0, keepdims=True) * (1.0 / D)
        xc = xt - m
        v = jnp.sum(xc * xc, axis=0, keepdims=True) * (1.0 / D)
        r = lax.rsqrt(v + EPS)
        xn = xc * r
        r2 = lax.rsqrt(v * (r * r) + EPS)
        xnT[:, al(i, TC)] = xn.astype(bf16)
        hT[:, al(i, TC)] = (xn * r2).astype(bf16)
        return 0

    lax.fori_loop(0, NX, ln_body, 0)
    for cp in g_copies(1):
        cp.start()
    w1_copy(1).start()

    lane = lax.broadcasted_iota(jnp.int32, (16, C), 1)
    sgn = 1.0 - 2.0 * (lax.broadcasted_iota(jnp.int32, (PR, C), 1) & 1).astype(f32)

    def kv_stage(g):
        r0 = g * RG if isinstance(g, int) else pl.multiple_of(g * RG, RG)
        for sb in range(RG // 16):
            rows = pl.ds(r0 + sb * 16, 16)
            w = [wsh[j, rows, :] for j in range(KS)]
            prev = None
            for t in range(NB):
                kc = kbuf[rows, t * C:(t + 1) * C].astype(f32)
                rolled = [pltpu.roll(kc, j, axis=1) for j in range(1, KS)]
                acc = kc * w[0]
                for j in range(1, KS):
                    if prev is None:
                        shifted = jnp.where(lane < j, 0.0, rolled[j - 1])
                    else:
                        shifted = jnp.where(lane < j, prev[j - 1], rolled[j - 1])
                    acc = acc + shifted * w[j]
                prev = rolled
                kv = acc * vbuf[rows, t * C:(t + 1) * C].astype(f32)
                kvs[t * RG + sb * 16:t * RG + (sb + 1) * 16, :] = kv.astype(bf16)

    def dft_stage(g):
        r0 = g * RG if isinstance(g, int) else pl.multiple_of(g * RG, RG)
        xf[...] = jnp.dot(kvs[...], fw_ref[...], preferred_element_type=f32)
        lk = jnp.concatenate(
            [skbuf[pl.ds(r0, RG), m * C:(m + 1) * C] for m in range(NB)], axis=0)
        kf[...] = jnp.dot(lk, fw_ref[...], preferred_element_type=f32)

    def idft_stage(g):
        r0 = g * RG if isinstance(g, int) else pl.multiple_of(g * RG, RG)
        y = jnp.dot(zb[...], iv_ref[...], preferred_element_type=f32)
        for i in range(NB):
            q = xnT[pl.ds(r0, RG), i * C:(i + 1) * C].astype(f32)
            sT[pl.ds(r0, RG), i * C:(i + 1) * C] = q * y[i * RG:(i + 1) * RG, :]

    def mac_stage(g):
        r0 = g * RG if isinstance(g, int) else pl.multiple_of(g * RG, RG)
        zero = zmask[...]

        def after(val, prev):
            bits = pltpu.bitcast(val, jnp.int32) | (pltpu.bitcast(prev, jnp.int32) & zero)
            return pltpu.bitcast(bits, f32)

        link = None
        for pr in range(RG // PR):
            def ld(ref, j, half, pr=pr):
                return ref[j * RG + pr * PR:j * RG + (pr + 1) * PR, half * C:(half + 1) * C]
            dd = dcol[pl.ds(r0 + pr * PR, PR), :]
            kr_prev = ki_prev = None
            for m in range(NB):
                kr, ki = ld(kf, m, 0), ld(kf, m, 1)
                if m == 0:
                    kr = kr + dd
                    cc, dm = kr, ki
                else:
                    cc = kr - sgn * ki_prev
                    dm = ki + sgn * kr_prev
                kr_prev, ki_prev = kr, ki
                pk[0, m] = cc
                pk[1, m] = dm - cc
                pk[2, m] = cc + dm
            for j in range(NB):
                px[j] = ld(xf, j, 0) + ld(xf, j, 1)
            for i0 in range(0, NB, IB):
                acc = [[None] * 3 for _ in range(IB)]
                kc = {}
                for j in range(i0 + IB):
                    a, b_, ab = ld(xf, j, 0), ld(xf, j, 1), px[j]
                    for t in range(IB):
                        m = i0 + t - j
                        if m < 0:
                            continue
                        if m not in kc:
                            kc[m] = (pk[0, m], pk[1, m], pk[2, m])
                        k0, k1, k2 = kc[m]
                        ps = (k0 * ab, a * k1, b_ * k2)
                        for q in range(3):
                            if acc[t][q] is not None:
                                acc[t][q] = acc[t][q] + ps[q]
                            elif link is None:
                                acc[t][q] = ps[q]
                            else:
                                acc[t][q] = after(ps[q], link[t][q])
                    kc = {m: val for m, val in kc.items() if m >= i0 - j}
                link = acc
                for t in range(IB):
                    s1, s2, s3 = acc[t]
                    rows = slice((i0 + t) * RG + pr * PR, (i0 + t) * RG + (pr + 1) * PR)
                    zb[rows, 0:C] = (s1 - s3).astype(bf16)
                    zb[rows, C:2 * C] = (s1 + s2).astype(bf16)

    for cp in g_copies(0):
        cp.wait()
    kv_stage(0)
    dft_stage(0)

    def p1_body(c, _):
        @pl.when(c + 2 < N1)
        def _():
            for cp in g_copies(c + 2):
                cp.start()
            w1_copy(c + 2).start()

        @pl.when(c + 2 >= N1)
        def _():
            w2_copy(c + 2 - N1).start()

        @pl.when(c + 1 < N1)
        def _():
            for cp in g_copies(c + 1):
                cp.wait()

        w1_copy(c).wait()
        idft_stage(jnp.maximum(c - 1, 0))
        mac_stage(c)
        gn = jnp.minimum(c + 1, N1 - 1)
        kv_stage(gn)
        dft_stage(gn)
        u = jnp.dot(hT[...], w1buf[c], preferred_element_type=f32)
        nt = FC // C
        b1c = b1s[pl.ds(c * nt, nt), :]
        u = u + jnp.concatenate([b1c[t:t + 1, :] for t in range(nt)], axis=1)
        ubuf[c] = _gelu(u).astype(bf16)
        return 0

    lax.fori_loop(0, N1, p1_body, 0, unroll=3)
    idft_stage(N1 - 1)

    def p2_body(p, _):
        @pl.when(p + 2 < N2)
        def _():
            w2_copy(p + 2).start()

        w2_copy(p).wait()
        acc = jnp.dot(ubuf[0], w2buf[p, 0:FC, :], preferred_element_type=f32)
        for c in range(1, N1):
            acc = acc + jnp.dot(ubuf[c], w2buf[p, c * FC:(c + 1) * FC, :],
                                preferred_element_type=f32)
        nt = SC // C
        b2c = b2s[pl.ds(p * nt, nt), :]
        y = acc + jnp.concatenate([b2c[t:t + 1, :] for t in range(nt)], axis=1)
        g = y * jax.nn.sigmoid(y)
        obuf[:, al(p, SC)] = (xbuf[:, al(p, SC)].astype(f32) + sT[:, al(p, SC)] * g).astype(bf16)
        o_copy(p).start()
        return 0

    lax.fori_loop(0, N2, p2_body, 0)
    for p in range(N2):
        o_copy(p).wait()


def pallas_recurrent_scan__ssm_conv_h3__mixer_token_mlp__prompt_kernel(
    A_q: jax.Array,
    A_k: jax.Array,
    A_v: jax.Array,
    A_shift_k: jax.Array,
    A_ssm_k: jax.Array,
    A_ssm_D: jax.Array,
    B_x: jax.Array,
    B_w1: jax.Array,
    B_b1: jax.Array,
    B_w2: jax.Array,
    B_b2: jax.Array,
):
    del B_x
    fw, iv = _dft_mats()
    hbm_spec = pl.BlockSpec(memory_space=pltpu.HBM)
    vmem_spec = pl.BlockSpec(memory_space=pltpu.VMEM)
    out = pl.pallas_call(
        _kernel,
        out_shape=jax.ShapeDtypeStruct((D, S), bf16),
        in_specs=[hbm_spec] * 6 + [vmem_spec] * 6,
        out_specs=hbm_spec,
        scratch_shapes=[
            pltpu.VMEM((D, S), bf16),
            pltpu.VMEM((D, S), bf16),
            pltpu.VMEM((D, S), bf16),
            pltpu.VMEM((D, S), bf16),
            pltpu.VMEM((N1, S, FC), bf16),
            pltpu.VMEM((N2, F, SC), bf16),
            pltpu.VMEM((D, S), bf16),
            pltpu.VMEM((D, S), bf16),
            pltpu.VMEM((D, S), bf16),
            pltpu.VMEM((NB * RG, C), bf16),
            pltpu.VMEM((N1, D, FC), bf16),
            pltpu.VMEM((D, S), f32),
            pltpu.VMEM((NB * RG, 2 * C), f32),
            pltpu.VMEM((NB * RG, 2 * C), f32),
            pltpu.VMEM((3, NB, PR, C), f32),
            pltpu.VMEM((NB, PR, C), f32),
            pltpu.VMEM((NB * RG, 2 * C), bf16),
            pltpu.VMEM((D, C), f32),
            pltpu.VMEM((KS, D, C), f32),
            pltpu.VMEM((F // C, C), f32),
            pltpu.VMEM((S // C, C), f32),
            pltpu.VMEM((PR, C), jnp.int32),
            pltpu.SemaphoreType.DMA((NX,)),
            pltpu.SemaphoreType.DMA((3, N1)),
            pltpu.SemaphoreType.DMA((N1,)),
            pltpu.SemaphoreType.DMA((N2,)),
            pltpu.SemaphoreType.DMA((N2,)),
        ],
        compiler_params=pltpu.CompilerParams(vmem_limit_bytes=110 * 1024 * 1024),
    )(
        A_q.reshape(S, D).T, A_k.reshape(S, D).T, A_v.reshape(S, D).T, A_ssm_k, B_w1, B_w2,
        A_shift_k.T, A_ssm_D, B_b1.reshape(F // C, C), B_b2.reshape(S // C, C),
        jnp.asarray(fw, bf16), jnp.asarray(iv, bf16),
    )
    return out.T.reshape(1, S, D)
```

```python
import jax
import jax.numpy as jnp
import numpy as np
from jax import lax
import jax.experimental.pallas as pl
import jax.experimental.pallas.tpu as pltpu

S, D, F, KS = 2048, 576, 4608, 4
C = 128
NB = S // C
FC = 512
N1 = F // FC
RG = D // N1
SC = 256
N2 = S // SC
TC = 256
NX = S // TC
XD = 4
PR = 8
IB = 2
EPS = 1e-5

f32 = jnp.float32
bf16 = jnp.bfloat16


def _dft_mats():
    t = np.arange(C, dtype=np.float64)
    th = 2.0 * np.pi * (np.arange(C, dtype=np.float64) + 0.5) / (2 * C)
    fw = np.concatenate([np.cos(np.outer(t, th)), -np.sin(np.outer(t, th))], axis=1)
    iv = np.concatenate([np.cos(np.outer(th, t)), -np.sin(np.outer(th, t))], axis=0) / C
    return fw.astype(np.float32), iv.astype(np.float32)


def _gelu(x):
    c = 0.7978845608028654
    hx = 0.5 * x
    return hx + hx * jnp.tanh(x * (c + (c * 0.044715) * (x * x)))


def _kernel(x_hbm, k_hbm, v_hbm, sk_hbm, w1_hbm, w2_hbm,
            shift_ref, d_ref, b1_ref, b2_ref, fw_ref, iv_ref,
            o_hbm,
            xbuf, kbuf, vbuf, skbuf, w1buf, w2buf, obuf,
            hT, xnT, kvs, ubuf, sT, xf, kf, pk, px, zb, dcol, wsh, b1s, b2s, zmask,
            sem_x, sem_g, sem_w1, sem_w2, sem_o):
    def al(i, n):
        return pl.ds(i * n if isinstance(i, int) else pl.multiple_of(i * n, n), n)

    def x_copy(i):
        return pltpu.make_async_copy(x_hbm.at[:, al(i, S // XD)], xbuf.at[:, al(i, S // XD)],
                                     sem_x.at[i])

    def g_copies(g):
        return [pltpu.make_async_copy(src.at[al(g, RG), :], dst.at[al(g, RG), :], sem_g.at[n, g])
                for n, (src, dst) in enumerate(((k_hbm, kbuf), (v_hbm, vbuf), (sk_hbm, skbuf)))]

    def w1_copy(c):
        return pltpu.make_async_copy(w1_hbm.at[:, al(c, FC)], w1buf.at[c], sem_w1.at[c])

    def w2_copy(p):
        return pltpu.make_async_copy(w2_hbm.at[:, al(p, SC)], w2buf.at[p], sem_w2.at[p])

    def o_copy(p):
        return pltpu.make_async_copy(obuf.at[:, al(p, SC)], o_hbm.at[:, al(p, SC)], sem_o.at[p])

    for i in range(XD):
        x_copy(i).start()
    for cp in g_copies(0) + g_copies(1):
        cp.start()
    w1_copy(0).start()

    dcol[...] = jnp.broadcast_to(d_ref[...].astype(f32).reshape(1, D), (C, D)).T
    sh = shift_ref[...].astype(f32)
    for j in range(KS):
        wsh[j] = jnp.broadcast_to(sh[j:j + 1, :], (C, D)).T
    b1s[...] = b1_ref[...].astype(f32)
    b2s[...] = b2_ref[...].astype(f32)
    zb[...] = jnp.zeros(zb.shape, bf16)
    zmask[...] = jnp.zeros(zmask.shape, jnp.int32)

    def ln_body(i, _):
        @pl.when(i % (NX // XD) == 0)
        def _():
            x_copy(i // (NX // XD)).wait()

        xt = xbuf[:, al(i, TC)].astype(f32)
        m = jnp.sum(xt, axis=0, keepdims=True) * (1.0 / D)
        xc = xt - m
        v = jnp.sum(xc * xc, axis=0, keepdims=True) * (1.0 / D)
        r = lax.rsqrt(v + EPS)
        xn = xc * r
        r2 = lax.rsqrt(v * (r * r) + EPS)
        xnT[:, al(i, TC)] = xn.astype(bf16)
        hT[:, al(i, TC)] = (xn * r2).astype(bf16)
        return 0

    lax.fori_loop(0, NX, ln_body, 0)

    lane = lax.broadcasted_iota(jnp.int32, (16, C), 1)
    sgn = 1.0 - 2.0 * (lax.broadcasted_iota(jnp.int32, (PR, C), 1) & 1).astype(f32)

    def kv_stage(g):
        r0 = g * RG if isinstance(g, int) else pl.multiple_of(g * RG, RG)
        for sb in range(RG // 16):
            rows = pl.ds(r0 + sb * 16, 16)
            w = [wsh[j, rows, :] for j in range(KS)]
            prev = None
            for t in range(NB):
                kc = kbuf[rows, t * C:(t + 1) * C].astype(f32)
                rolled = [pltpu.roll(kc, j, axis=1) for j in range(1, KS)]
                acc = kc * w[0]
                for j in range(1, KS):
                    if prev is None:
                        shifted = jnp.where(lane < j, 0.0, rolled[j - 1])
                    else:
                        shifted = jnp.where(lane < j, prev[j - 1], rolled[j - 1])
                    acc = acc + shifted * w[j]
                prev = rolled
                kv = acc * vbuf[rows, t * C:(t + 1) * C].astype(f32)
                kvs[t * RG + sb * 16:t * RG + (sb + 1) * 16, :] = kv.astype(bf16)

    def dft_stage(g):
        r0 = g * RG if isinstance(g, int) else pl.multiple_of(g * RG, RG)
        xf[...] = jnp.dot(kvs[...], fw_ref[...], preferred_element_type=f32)
        lk = jnp.concatenate(
            [skbuf[pl.ds(r0, RG), m * C:(m + 1) * C] for m in range(NB)], axis=0)
        kf[...] = jnp.dot(lk, fw_ref[...], preferred_element_type=f32)

    def idft_stage(g):
        r0 = g * RG if isinstance(g, int) else pl.multiple_of(g * RG, RG)
        y = jnp.dot(zb[...], iv_ref[...], preferred_element_type=f32)
        for i in range(NB):
            q = xnT[pl.ds(r0, RG), i * C:(i + 1) * C].astype(f32)
            sT[pl.ds(r0, RG), i * C:(i + 1) * C] = q * y[i * RG:(i + 1) * RG, :]

    def mac_stage(g):
        r0 = g * RG if isinstance(g, int) else pl.multiple_of(g * RG, RG)
        zero = zmask[...]

        def after(val, prev):
            bits = pltpu.bitcast(val, jnp.int32) | (pltpu.bitcast(prev, jnp.int32) & zero)
            return pltpu.bitcast(bits, f32)

        link = None
        for pr in range(RG // PR):
            def ld(ref, j, half, pr=pr):
                return ref[j * RG + pr * PR:j * RG + (pr + 1) * PR, half * C:(half + 1) * C]
            dd = dcol[pl.ds(r0 + pr * PR, PR), :]
            kr_prev = ki_prev = None
            for m in range(NB):
                kr, ki = ld(kf, m, 0), ld(kf, m, 1)
                if m == 0:
                    kr = kr + dd
                    cc, dm = kr, ki
                else:
                    cc = kr - sgn * ki_prev
                    dm = ki + sgn * kr_prev
                kr_prev, ki_prev = kr, ki
                pk[0, m] = cc
                pk[1, m] = dm - cc
                pk[2, m] = cc + dm
            for j in range(NB):
                px[j] = ld(xf, j, 0) + ld(xf, j, 1)
            for i0 in range(0, NB, IB):
                acc = [[None] * 3 for _ in range(IB)]
                kc = {}
                for j in range(i0 + IB):
                    a, b_, ab = ld(xf, j, 0), ld(xf, j, 1), px[j]
                    for t in range(IB):
                        m = i0 + t - j
                        if m < 0:
                            continue
                        if m not in kc:
                            kc[m] = (pk[0, m], pk[1, m], pk[2, m])
                        k0, k1, k2 = kc[m]
                        ps = (k0 * ab, a * k1, b_ * k2)
                        for q in range(3):
                            if acc[t][q] is not None:
                                acc[t][q] = acc[t][q] + ps[q]
                            elif link is None:
                                acc[t][q] = ps[q]
                            else:
                                acc[t][q] = after(ps[q], link[t][q])
                    kc = {m: val for m, val in kc.items() if m >= i0 - j}
                link = acc
                for t in range(IB):
                    s1, s2, s3 = acc[t]
                    rows = slice((i0 + t) * RG + pr * PR, (i0 + t) * RG + (pr + 1) * PR)
                    zb[rows, 0:C] = (s1 - s3).astype(bf16)
                    zb[rows, C:2 * C] = (s1 + s2).astype(bf16)

    for cp in g_copies(0):
        cp.wait()
    kv_stage(0)
    dft_stage(0)

    def p1_body(c, _):
        w1_copy(c).wait()

        @pl.when(c + 1 < N1)
        def _():
            for cp in g_copies(c + 1):
                cp.wait()
            w1_copy(c + 1).start()

        @pl.when(c + 2 < N1)
        def _():
            for cp in g_copies(c + 2):
                cp.start()

        @pl.when(c + 2 >= N1)
        def _():
            w2_copy(c + 2 - N1).start()

        idft_stage(jnp.maximum(c - 1, 0))
        mac_stage(c)
        gn = jnp.minimum(c + 1, N1 - 1)
        kv_stage(gn)
        dft_stage(gn)
        u = jnp.dot(hT[...], w1buf[c], preferred_element_type=f32)
        nt = FC // C
        b1c = b1s[pl.ds(c * nt, nt), :]
        u = u + jnp.concatenate([b1c[t:t + 1, :] for t in range(nt)], axis=1)
        ubuf[c] = _gelu(u).astype(bf16)
        return 0

    lax.fori_loop(0, N1, p1_body, 0, unroll=3)
    idft_stage(N1 - 1)

    def p2_body(p, _):
        @pl.when(p + 2 < N2)
        def _():
            w2_copy(p + 2).start()

        w2_copy(p).wait()
        acc = jnp.dot(ubuf[0], w2buf[p, 0:FC, :], preferred_element_type=f32)
        for c in range(1, N1):
            acc = acc + jnp.dot(ubuf[c], w2buf[p, c * FC:(c + 1) * FC, :],
                                preferred_element_type=f32)
        nt = SC // C
        b2c = b2s[pl.ds(p * nt, nt), :]
        y = acc + jnp.concatenate([b2c[t:t + 1, :] for t in range(nt)], axis=1)
        g = y * jax.nn.sigmoid(y)
        obuf[:, al(p, SC)] = (xbuf[:, al(p, SC)].astype(f32) + sT[:, al(p, SC)] * g).astype(bf16)
        o_copy(p).start()
        return 0

    lax.fori_loop(0, N2, p2_body, 0)
    for p in range(N2):
        o_copy(p).wait()


def pallas_recurrent_scan__ssm_conv_h3__mixer_token_mlp__prompt_kernel(
    A_q: jax.Array,
    A_k: jax.Array,
    A_v: jax.Array,
    A_shift_k: jax.Array,
    A_ssm_k: jax.Array,
    A_ssm_D: jax.Array,
    B_x: jax.Array,
    B_w1: jax.Array,
    B_b1: jax.Array,
    B_w2: jax.Array,
    B_b2: jax.Array,
):
    del B_x
    fw, iv = _dft_mats()
    hbm_spec = pl.BlockSpec(memory_space=pltpu.HBM)
    vmem_spec = pl.BlockSpec(memory_space=pltpu.VMEM)
    out = pl.pallas_call(
        _kernel,
        out_shape=jax.ShapeDtypeStruct((D, S), bf16),
        in_specs=[hbm_spec] * 6 + [vmem_spec] * 6,
        out_specs=hbm_spec,
        scratch_shapes=[
            pltpu.VMEM((D, S), bf16),
            pltpu.VMEM((D, S), bf16),
            pltpu.VMEM((D, S), bf16),
            pltpu.VMEM((D, S), bf16),
            pltpu.VMEM((N1, S, FC), bf16),
            pltpu.VMEM((N2, F, SC), bf16),
            pltpu.VMEM((D, S), bf16),
            pltpu.VMEM((D, S), bf16),
            pltpu.VMEM((D, S), bf16),
            pltpu.VMEM((NB * RG, C), bf16),
            pltpu.VMEM((N1, D, FC), bf16),
            pltpu.VMEM((D, S), f32),
            pltpu.VMEM((NB * RG, 2 * C), f32),
            pltpu.VMEM((NB * RG, 2 * C), f32),
            pltpu.VMEM((3, NB, PR, C), f32),
            pltpu.VMEM((NB, PR, C), f32),
            pltpu.VMEM((NB * RG, 2 * C), bf16),
            pltpu.VMEM((D, C), f32),
            pltpu.VMEM((KS, D, C), f32),
            pltpu.VMEM((F // C, C), f32),
            pltpu.VMEM((S // C, C), f32),
            pltpu.VMEM((PR, C), jnp.int32),
            pltpu.SemaphoreType.DMA((XD,)),
            pltpu.SemaphoreType.DMA((3, N1)),
            pltpu.SemaphoreType.DMA((N1,)),
            pltpu.SemaphoreType.DMA((N2,)),
            pltpu.SemaphoreType.DMA((N2,)),
        ],
        compiler_params=pltpu.CompilerParams(vmem_limit_bytes=110 * 1024 * 1024),
    )(
        A_q.reshape(S, D).T, A_k.reshape(S, D).T, A_v.reshape(S, D).T, A_ssm_k, B_w1, B_w2,
        A_shift_k.T, A_ssm_D, B_b1.reshape(F // C, C), B_b2.reshape(S // C, C),
        jnp.asarray(fw, bf16), jnp.asarray(iv, bf16),
    )
    return out.T.reshape(1, S, D)
```

```python
import jax
import jax.numpy as jnp
import numpy as np
from jax import lax
import jax.experimental.pallas as pl
import jax.experimental.pallas.tpu as pltpu

S, D, F, KS = 2048, 576, 4608, 4
C = 128
NB = S // C
FC = 512
N1 = F // FC
RG = D // N1
SC = 512
N2 = S // SC
OC = 128
TC = 256
NX = S // TC
XD = 4
PR = 8
IB = 2
EPS = 1e-5

f32 = jnp.float32
bf16 = jnp.bfloat16


def _dft_mats():
    t = np.arange(C, dtype=np.float64)
    th = 2.0 * np.pi * (np.arange(C, dtype=np.float64) + 0.5) / (2 * C)
    fw = np.concatenate([np.cos(np.outer(t, th)), -np.sin(np.outer(t, th))], axis=1)
    iv = np.concatenate([np.cos(np.outer(th, t)), -np.sin(np.outer(th, t))], axis=0) / C
    return fw.astype(np.float32), iv.astype(np.float32)


def _gelu(x):
    c = 0.7978845608028654
    hx = 0.5 * x
    return hx + hx * jnp.tanh(x * (c + (c * 0.044715) * (x * x)))


def _kernel(x_hbm, k_hbm, v_hbm, sk_hbm, w1_hbm, w2_hbm,
            shift_ref, d_ref, b1_ref, b2_ref, fw_ref, iv_ref,
            o_hbm,
            xbuf, kbuf, vbuf, skbuf, w1buf, w2buf, obuf,
            hT, xnT, kvs, ubuf, sT, xf, kf, pk, px, zb, dcol, wsh, b1s, b2s, zmask,
            sem_x, sem_g, sem_w1, sem_w2, sem_o):
    def al(i, n):
        return pl.ds(i * n if isinstance(i, int) else pl.multiple_of(i * n, n), n)

    def x_copy(i):
        return pltpu.make_async_copy(x_hbm.at[:, al(i, S // XD)], xbuf.at[:, al(i, S // XD)],
                                     sem_x.at[i])

    def g_copies(g):
        return [pltpu.make_async_copy(src.at[al(g, RG), :], dst.at[al(g, RG), :], sem_g.at[n, g])
                for n, (src, dst) in enumerate(((k_hbm, kbuf), (v_hbm, vbuf), (sk_hbm, skbuf)))]

    def w1_copy(c):
        return pltpu.make_async_copy(w1_hbm.at[:, al(c, FC)], w1buf.at[c], sem_w1.at[c])

    def w2_copy(p):
        return pltpu.make_async_copy(w2_hbm.at[:, al(p, SC)], w2buf.at[p], sem_w2.at[p])

    def o_copy(h):
        return pltpu.make_async_copy(obuf.at[:, al(h, OC)], o_hbm.at[:, al(h, OC)], sem_o.at[h])

    for i in range(XD):
        x_copy(i).start()
    for cp in g_copies(0) + g_copies(1):
        cp.start()
    w1_copy(0).start()

    dcol[...] = jnp.broadcast_to(d_ref[...].astype(f32).reshape(1, D), (C, D)).T
    sh = shift_ref[...].astype(f32)
    for j in range(KS):
        wsh[j] = jnp.broadcast_to(sh[j:j + 1, :], (C, D)).T
    b1s[...] = b1_ref[...].astype(f32)
    b2s[...] = b2_ref[...].astype(f32)
    zb[...] = jnp.zeros(zb.shape, bf16)
    zmask[...] = jnp.zeros(zmask.shape, jnp.int32)

    def ln_body(i, _):
        @pl.when(i % (NX // XD) == 0)
        def _():
            x_copy(i // (NX // XD)).wait()

        xt = xbuf[:, al(i, TC)].astype(f32)
        m = jnp.sum(xt, axis=0, keepdims=True) * (1.0 / D)
        xc = xt - m
        v = jnp.sum(xc * xc, axis=0, keepdims=True) * (1.0 / D)
        r = lax.rsqrt(v + EPS)
        xn = xc * r
        r2 = lax.rsqrt(v * (r * r) + EPS)
        xnT[:, al(i, TC)] = xn.astype(bf16)
        hT[:, al(i, TC)] = (xn * r2).astype(bf16)
        return 0

    lax.fori_loop(0, NX, ln_body, 0)

    lane = lax.broadcasted_iota(jnp.int32, (16, C), 1)
    sgn = 1.0 - 2.0 * (lax.broadcasted_iota(jnp.int32, (PR, C), 1) & 1).astype(f32)

    def kv_stage(g):
        r0 = g * RG if isinstance(g, int) else pl.multiple_of(g * RG, RG)
        for sb in range(RG // 16):
            rows = pl.ds(r0 + sb * 16, 16)
            w = [wsh[j, rows, :] for j in range(KS)]
            prev = None
            for t in range(NB):
                kc = kbuf[rows, t * C:(t + 1) * C].astype(f32)
                rolled = [pltpu.roll(kc, j, axis=1) for j in range(1, KS)]
                acc = kc * w[0]
                for j in range(1, KS):
                    if prev is None:
                        shifted = jnp.where(lane < j, 0.0, rolled[j - 1])
                    else:
                        shifted = jnp.where(lane < j, prev[j - 1], rolled[j - 1])
                    acc = acc + shifted * w[j]
                prev = rolled
                kv = acc * vbuf[rows, t * C:(t + 1) * C].astype(f32)
                kvs[t * RG + sb * 16:t * RG + (sb + 1) * 16, :] = kv.astype(bf16)

    def dft_stage(g):
        r0 = g * RG if isinstance(g, int) else pl.multiple_of(g * RG, RG)
        xf[...] = jnp.dot(kvs[...], fw_ref[...], preferred_element_type=f32)
        lk = jnp.concatenate(
            [skbuf[pl.ds(r0, RG), m * C:(m + 1) * C] for m in range(NB)], axis=0)
        kf[...] = jnp.dot(lk, fw_ref[...], preferred_element_type=f32)

    def idft_stage(g):
        r0 = g * RG if isinstance(g, int) else pl.multiple_of(g * RG, RG)
        y = jnp.dot(zb[...], iv_ref[...], preferred_element_type=f32)
        for i in range(NB):
            q = xnT[pl.ds(r0, RG), i * C:(i + 1) * C].astype(f32)
            sT[pl.ds(r0, RG), i * C:(i + 1) * C] = q * y[i * RG:(i + 1) * RG, :]

    def mac_stage(g):
        r0 = g * RG if isinstance(g, int) else pl.multiple_of(g * RG, RG)
        zero = zmask[...]

        def after(val, prev):
            bits = pltpu.bitcast(val, jnp.int32) | (pltpu.bitcast(prev, jnp.int32) & zero)
            return pltpu.bitcast(bits, f32)

        link = None
        for pr in range(RG // PR):
            def ld(ref, j, half, pr=pr):
                return ref[j * RG + pr * PR:j * RG + (pr + 1) * PR, half * C:(half + 1) * C]
            dd = dcol[pl.ds(r0 + pr * PR, PR), :]
            kr_prev = ki_prev = None
            for m in range(NB):
                kr, ki = ld(kf, m, 0), ld(kf, m, 1)
                if m == 0:
                    kr = kr + dd
                    cc, dm = kr, ki
                else:
                    cc = kr - sgn * ki_prev
                    dm = ki + sgn * kr_prev
                kr_prev, ki_prev = kr, ki
                pk[0, m] = cc
                pk[1, m] = dm - cc
                pk[2, m] = cc + dm
            for j in range(NB):
                px[j] = ld(xf, j, 0) + ld(xf, j, 1)
            for i0 in range(0, NB, IB):
                acc = [[None] * 3 for _ in range(IB)]
                kc = {}
                for j in range(i0 + IB):
                    a, b_, ab = ld(xf, j, 0), ld(xf, j, 1), px[j]
                    for t in range(IB):
                        m = i0 + t - j
                        if m < 0:
                            continue
                        if m not in kc:
                            kc[m] = (pk[0, m], pk[1, m], pk[2, m])
                        k0, k1, k2 = kc[m]
                        ps = (k0 * ab, a * k1, b_ * k2)
                        for q in range(3):
                            if acc[t][q] is not None:
                                acc[t][q] = acc[t][q] + ps[q]
                            elif link is None:
                                acc[t][q] = ps[q]
                            else:
                                acc[t][q] = after(ps[q], link[t][q])
                    kc = {m: val for m, val in kc.items() if m >= i0 - j}
                link = acc
                for t in range(IB):
                    s1, s2, s3 = acc[t]
                    rows = slice((i0 + t) * RG + pr * PR, (i0 + t) * RG + (pr + 1) * PR)
                    zb[rows, 0:C] = (s1 - s3).astype(bf16)
                    zb[rows, C:2 * C] = (s1 + s2).astype(bf16)

    for cp in g_copies(0):
        cp.wait()
    kv_stage(0)
    dft_stage(0)

    def p1_body(c, _):
        w1_copy(c).wait()

        @pl.when(c + 1 < N1)
        def _():
            for cp in g_copies(c + 1):
                cp.wait()
            w1_copy(c + 1).start()

        @pl.when(c + 2 < N1)
        def _():
            for cp in g_copies(c + 2):
                cp.start()

        @pl.when(c + 2 >= N1)
        def _():
            w2_copy(c + 2 - N1).start()

        idft_stage(jnp.maximum(c - 1, 0))
        mac_stage(c)
        gn = jnp.minimum(c + 1, N1 - 1)
        kv_stage(gn)
        dft_stage(gn)
        u = jnp.dot(hT[...], w1buf[c], preferred_element_type=f32)
        nt = FC // C
        b1c = b1s[pl.ds(c * nt, nt), :]
        u = u + jnp.concatenate([b1c[t:t + 1, :] for t in range(nt)], axis=1)
        ubuf[c] = _gelu(u).astype(bf16)
        return 0

    lax.fori_loop(0, N1, p1_body, 0, unroll=3)
    idft_stage(N1 - 1)

    def p2_body(p, _):
        @pl.when(p + 2 < N2)
        def _():
            w2_copy(p + 2).start()

        w2_copy(p).wait()
        acc = jnp.dot(ubuf[0], w2buf[p, 0:FC, :], preferred_element_type=f32)
        for c in range(1, N1):
            acc = acc + jnp.dot(ubuf[c], w2buf[p, c * FC:(c + 1) * FC, :],
                                preferred_element_type=f32)
        for h in range(SC // OC):
            oc = p * (SC // OC) + h
            nt = OC // C
            b2c = b2s[pl.ds(oc * nt, nt), :]
            y = acc[:, h * OC:(h + 1) * OC] + jnp.concatenate(
                [b2c[t:t + 1, :] for t in range(nt)], axis=1)
            g = y * jax.nn.sigmoid(y)
            obuf[:, al(oc, OC)] = (
                xbuf[:, al(oc, OC)].astype(f32) + sT[:, al(oc, OC)] * g).astype(bf16)
            o_copy(oc).start()
        return 0

    lax.fori_loop(0, N2, p2_body, 0)
    for h in range(S // OC):
        o_copy(h).wait()


def pallas_recurrent_scan__ssm_conv_h3__mixer_token_mlp__prompt_kernel(
    A_q: jax.Array,
    A_k: jax.Array,
    A_v: jax.Array,
    A_shift_k: jax.Array,
    A_ssm_k: jax.Array,
    A_ssm_D: jax.Array,
    B_x: jax.Array,
    B_w1: jax.Array,
    B_b1: jax.Array,
    B_w2: jax.Array,
    B_b2: jax.Array,
):
    del B_x
    fw, iv = _dft_mats()
    hbm_spec = pl.BlockSpec(memory_space=pltpu.HBM)
    vmem_spec = pl.BlockSpec(memory_space=pltpu.VMEM)
    out = pl.pallas_call(
        _kernel,
        out_shape=jax.ShapeDtypeStruct((D, S), bf16),
        in_specs=[hbm_spec] * 6 + [vmem_spec] * 6,
        out_specs=hbm_spec,
        scratch_shapes=[
            pltpu.VMEM((D, S), bf16),
            pltpu.VMEM((D, S), bf16),
            pltpu.VMEM((D, S), bf16),
            pltpu.VMEM((D, S), bf16),
            pltpu.VMEM((N1, S, FC), bf16),
            pltpu.VMEM((N2, F, SC), bf16),
            pltpu.VMEM((D, S), bf16),
            pltpu.VMEM((D, S), bf16),
            pltpu.VMEM((D, S), bf16),
            pltpu.VMEM((NB * RG, C), bf16),
            pltpu.VMEM((N1, D, FC), bf16),
            pltpu.VMEM((D, S), f32),
            pltpu.VMEM((NB * RG, 2 * C), f32),
            pltpu.VMEM((NB * RG, 2 * C), f32),
            pltpu.VMEM((3, NB, PR, C), f32),
            pltpu.VMEM((NB, PR, C), f32),
            pltpu.VMEM((NB * RG, 2 * C), bf16),
            pltpu.VMEM((D, C), f32),
            pltpu.VMEM((KS, D, C), f32),
            pltpu.VMEM((F // C, C), f32),
            pltpu.VMEM((S // C, C), f32),
            pltpu.VMEM((PR, C), jnp.int32),
            pltpu.SemaphoreType.DMA((XD,)),
            pltpu.SemaphoreType.DMA((3, N1)),
            pltpu.SemaphoreType.DMA((N1,)),
            pltpu.SemaphoreType.DMA((N2,)),
            pltpu.SemaphoreType.DMA((S // OC,)),
        ],
        compiler_params=pltpu.CompilerParams(vmem_limit_bytes=110 * 1024 * 1024),
    )(
        A_q.reshape(S, D).T, A_k.reshape(S, D).T, A_v.reshape(S, D).T, A_ssm_k, B_w1, B_w2,
        A_shift_k.T, A_ssm_D, B_b1.reshape(F // C, C), B_b2.reshape(S // C, C),
        jnp.asarray(fw, bf16), jnp.asarray(iv, bf16),
    )
    return out.T.reshape(1, S, D)
```

```python
import jax
import jax.numpy as jnp
import numpy as np
from jax import lax
import jax.experimental.pallas as pl
import jax.experimental.pallas.tpu as pltpu

S, D, F, KS = 2048, 576, 4608, 4
C = 128
NB = S // C
FC = 512
N1 = F // FC
RG = D // N1
SC = 512
N2 = S // SC
OC = 128
TC = 256
NX = S // TC
XD = 4
PR = 8
IB = 2
EPS = 1e-5

f32 = jnp.float32
bf16 = jnp.bfloat16


def _dft_mats():
    t = np.arange(C, dtype=np.float64)
    th = 2.0 * np.pi * (np.arange(C, dtype=np.float64) + 0.5) / (2 * C)
    fw = np.concatenate([np.cos(np.outer(t, th)), -np.sin(np.outer(t, th))], axis=1)
    iv = np.concatenate([np.cos(np.outer(th, t)), -np.sin(np.outer(th, t))], axis=0) / C
    return fw.astype(np.float32), iv.astype(np.float32)


def _gelu(x):
    c = 0.7978845608028654
    hx = 0.5 * x
    return hx + hx * jnp.tanh(x * (c + (c * 0.044715) * (x * x)))


def _kernel(x_hbm, k_hbm, v_hbm, sk_hbm, w1_hbm, w2_hbm,
            shift_ref, d_ref, b1_ref, b2_ref, fw_ref, iv_ref,
            o_hbm,
            xbuf, kbuf, vbuf, skbuf, w1buf, w2buf, obuf,
            hT, xnT, kvs, ubuf, sT, xf, kf, pk, px, zb, dcol, wsh, b1s, b2s, zmask,
            sem_x, sem_g, sem_w1, sem_w2, sem_o):
    def al(i, n):
        return pl.ds(i * n if isinstance(i, int) else pl.multiple_of(i * n, n), n)

    def x_copy(i):
        return pltpu.make_async_copy(x_hbm.at[:, al(i, S // XD)], xbuf.at[:, al(i, S // XD)],
                                     sem_x.at[i])

    def g_copies(g):
        return [pltpu.make_async_copy(src.at[al(g, RG), :], dst.at[al(g, RG), :], sem_g.at[n, g])
                for n, (src, dst) in enumerate(((k_hbm, kbuf), (v_hbm, vbuf), (sk_hbm, skbuf)))]

    def w1_copy(c):
        return pltpu.make_async_copy(w1_hbm.at[:, al(c, FC)], w1buf.at[c], sem_w1.at[c])

    def w2_copy(p):
        return pltpu.make_async_copy(w2_hbm.at[:, al(p, SC)], w2buf.at[p], sem_w2.at[p])

    def o_copy(h):
        return pltpu.make_async_copy(obuf.at[:, al(h, OC)], o_hbm.at[:, al(h, OC)], sem_o.at[h])

    for i in range(XD):
        x_copy(i).start()
    for cp in g_copies(0) + g_copies(1):
        cp.start()
    w1_copy(0).start()

    dcol[...] = jnp.broadcast_to(d_ref[...].astype(f32).reshape(1, D), (C, D)).T
    sh = shift_ref[...].astype(f32)
    for j in range(KS):
        wsh[j] = jnp.broadcast_to(sh[j:j + 1, :], (C, D)).T
    b1s[...] = b1_ref[...].astype(f32)
    b2s[...] = b2_ref[...].astype(f32)
    zb[...] = jnp.zeros(zb.shape, bf16)
    zmask[...] = jnp.zeros(zmask.shape, jnp.int32)

    def ln_body(i, _):
        @pl.when(i % (NX // XD) == 0)
        def _():
            x_copy(i // (NX // XD)).wait()

        xt = xbuf[:, al(i, TC)].astype(f32)
        m = jnp.sum(xt, axis=0, keepdims=True) * (1.0 / D)
        xc = xt - m
        v = jnp.sum(xc * xc, axis=0, keepdims=True) * (1.0 / D)
        r = lax.rsqrt(v + EPS)
        xn = xc * r
        r2 = lax.rsqrt(v * (r * r) + EPS)
        xnT[:, al(i, TC)] = xn.astype(bf16)
        hT[:, al(i, TC)] = (xn * r2).astype(bf16)
        return 0

    lax.fori_loop(0, NX, ln_body, 0)

    lane = lax.broadcasted_iota(jnp.int32, (16, C), 1)
    sgn = 1.0 - 2.0 * (lax.broadcasted_iota(jnp.int32, (PR, C), 1) & 1).astype(f32)

    def kv_stage(g):
        r0 = g * RG if isinstance(g, int) else pl.multiple_of(g * RG, RG)
        for sb in range(RG // 16):
            rows = pl.ds(r0 + sb * 16, 16)
            w = [wsh[j, rows, :] for j in range(KS)]
            prev = None
            for t in range(NB):
                kc = kbuf[rows, t * C:(t + 1) * C].astype(f32)
                rolled = [pltpu.roll(kc, j, axis=1) for j in range(1, KS)]
                acc = kc * w[0]
                for j in range(1, KS):
                    if prev is None:
                        shifted = jnp.where(lane < j, 0.0, rolled[j - 1])
                    else:
                        shifted = jnp.where(lane < j, prev[j - 1], rolled[j - 1])
                    acc = acc + shifted * w[j]
                prev = rolled
                kv = acc * vbuf[rows, t * C:(t + 1) * C].astype(f32)
                kvs[t * RG + sb * 16:t * RG + (sb + 1) * 16, :] = kv.astype(bf16)

    def dft_stage(g):
        r0 = g * RG if isinstance(g, int) else pl.multiple_of(g * RG, RG)
        xf[...] = jnp.dot(kvs[...], fw_ref[...], preferred_element_type=f32)
        lk = jnp.concatenate(
            [skbuf[pl.ds(r0, RG), m * C:(m + 1) * C] for m in range(NB)], axis=0)
        kf[...] = jnp.dot(lk, fw_ref[...], preferred_element_type=f32)

    def idft_stage(g):
        r0 = g * RG if isinstance(g, int) else pl.multiple_of(g * RG, RG)
        y = jnp.dot(zb[...], iv_ref[...], preferred_element_type=f32)
        for i in range(NB):
            q = xnT[pl.ds(r0, RG), i * C:(i + 1) * C].astype(f32)
            sT[pl.ds(r0, RG), i * C:(i + 1) * C] = q * y[i * RG:(i + 1) * RG, :]

    def mac_stage(g):
        r0 = g * RG if isinstance(g, int) else pl.multiple_of(g * RG, RG)
        zero = zmask[...]

        def after(val, prev):
            bits = pltpu.bitcast(val, jnp.int32) | (pltpu.bitcast(prev, jnp.int32) & zero)
            return pltpu.bitcast(bits, f32)

        link = None
        for pr in range(RG // PR):
            def ld(ref, j, half, pr=pr):
                return ref[j * RG + pr * PR:j * RG + (pr + 1) * PR, half * C:(half + 1) * C]
            dd = dcol[pl.ds(r0 + pr * PR, PR), :]
            kr_prev = ki_prev = None
            for m in range(NB):
                kr, ki = ld(kf, m, 0), ld(kf, m, 1)
                if m == 0:
                    kr = kr + dd
                    cc, dm = kr, ki
                else:
                    cc = kr - sgn * ki_prev
                    dm = ki + sgn * kr_prev
                kr_prev, ki_prev = kr, ki
                pk[0, m] = cc
                pk[1, m] = dm - cc
                pk[2, m] = cc + dm
            for j in range(NB):
                px[j] = ld(xf, j, 0) + ld(xf, j, 1)
            for i0 in range(0, NB, IB):
                acc = [[None] * 3 for _ in range(IB)]
                kc = {}
                for j in range(i0 + IB):
                    a, b_, ab = ld(xf, j, 0), ld(xf, j, 1), px[j]
                    for t in range(IB):
                        m = i0 + t - j
                        if m < 0:
                            continue
                        if m not in kc:
                            kc[m] = (pk[0, m], pk[1, m], pk[2, m])
                        k0, k1, k2 = kc[m]
                        ps = (k0 * ab, a * k1, b_ * k2)
                        for q in range(3):
                            if acc[t][q] is not None:
                                acc[t][q] = acc[t][q] + ps[q]
                            elif link is None:
                                acc[t][q] = ps[q]
                            else:
                                acc[t][q] = after(ps[q], link[t][q])
                    kc = {m: val for m, val in kc.items() if m >= i0 - j}
                link = acc
                for t in range(IB):
                    s1, s2, s3 = acc[t]
                    rows = slice((i0 + t) * RG + pr * PR, (i0 + t) * RG + (pr + 1) * PR)
                    zb[rows, 0:C] = (s1 - s3).astype(bf16)
                    zb[rows, C:2 * C] = (s1 + s2).astype(bf16)

    for cp in g_copies(0):
        cp.wait()
    kv_stage(0)
    dft_stage(0)

    def p1_body(c, _):
        w1_copy(c).wait()

        @pl.when(c + 1 < N1)
        def _():
            for cp in g_copies(c + 1):
                cp.wait()
            w1_copy(c + 1).start()

        @pl.when(c + 2 < N1)
        def _():
            for cp in g_copies(c + 2):
                cp.start()

        @pl.when(c + 2 >= N1)
        def _():
            w2_copy(c + 2 - N1).start()

        idft_stage(jnp.maximum(c - 1, 0))
        mac_stage(c)
        gn = jnp.minimum(c + 1, N1 - 1)
        kv_stage(gn)
        dft_stage(gn)
        u = jnp.dot(hT[:, 0:512], w1buf[c, 0:512, :], preferred_element_type=f32)
        for kk in range(1, 4):
            u = u + jnp.dot(hT[:, kk * 512:(kk + 1) * 512], w1buf[c, kk * 512:(kk + 1) * 512, :],
                            preferred_element_type=f32)
        for t in range(FC // C):
            cols = slice(t * C, (t + 1) * C)
            ut = u[:, cols] + b1s[pl.ds(c * (FC // C) + t, 1), :]
            ubuf[c, :, cols] = _gelu(ut).astype(bf16)
        return 0

    lax.fori_loop(0, N1, p1_body, 0, unroll=3)
    idft_stage(N1 - 1)

    def p2_body(p, _):
        @pl.when(p + 2 < N2)
        def _():
            w2_copy(p + 2).start()

        w2_copy(p).wait()
        acc = jnp.dot(ubuf[0], w2buf[p, 0:FC, :], preferred_element_type=f32)
        for c in range(1, N1):
            acc = acc + jnp.dot(ubuf[c], w2buf[p, c * FC:(c + 1) * FC, :],
                                preferred_element_type=f32)
        for h in range(SC // OC):
            oc = p * (SC // OC) + h
            nt = OC // C
            b2c = b2s[pl.ds(oc * nt, nt), :]
            y = acc[:, h * OC:(h + 1) * OC] + jnp.concatenate(
                [b2c[t:t + 1, :] for t in range(nt)], axis=1)
            g = y * jax.nn.sigmoid(y)
            obuf[:, al(oc, OC)] = (
                xbuf[:, al(oc, OC)].astype(f32) + sT[:, al(oc, OC)] * g).astype(bf16)
            o_copy(oc).start()
        return 0

    lax.fori_loop(0, N2, p2_body, 0)
    for h in range(S // OC):
        o_copy(h).wait()


def pallas_recurrent_scan__ssm_conv_h3__mixer_token_mlp__prompt_kernel(
    A_q: jax.Array,
    A_k: jax.Array,
    A_v: jax.Array,
    A_shift_k: jax.Array,
    A_ssm_k: jax.Array,
    A_ssm_D: jax.Array,
    B_x: jax.Array,
    B_w1: jax.Array,
    B_b1: jax.Array,
    B_w2: jax.Array,
    B_b2: jax.Array,
):
    del B_x
    fw, iv = _dft_mats()
    hbm_spec = pl.BlockSpec(memory_space=pltpu.HBM)
    vmem_spec = pl.BlockSpec(memory_space=pltpu.VMEM)
    out = pl.pallas_call(
        _kernel,
        out_shape=jax.ShapeDtypeStruct((D, S), bf16),
        in_specs=[hbm_spec] * 6 + [vmem_spec] * 6,
        out_specs=hbm_spec,
        scratch_shapes=[
            pltpu.VMEM((D, S), bf16),
            pltpu.VMEM((D, S), bf16),
            pltpu.VMEM((D, S), bf16),
            pltpu.VMEM((D, S), bf16),
            pltpu.VMEM((N1, S, FC), bf16),
            pltpu.VMEM((N2, F, SC), bf16),
            pltpu.VMEM((D, S), bf16),
            pltpu.VMEM((D, S), bf16),
            pltpu.VMEM((D, S), bf16),
            pltpu.VMEM((NB * RG, C), bf16),
            pltpu.VMEM((N1, D, FC), bf16),
            pltpu.VMEM((D, S), f32),
            pltpu.VMEM((NB * RG, 2 * C), f32),
            pltpu.VMEM((NB * RG, 2 * C), f32),
            pltpu.VMEM((3, NB, PR, C), f32),
            pltpu.VMEM((NB, PR, C), f32),
            pltpu.VMEM((NB * RG, 2 * C), bf16),
            pltpu.VMEM((D, C), f32),
            pltpu.VMEM((KS, D, C), f32),
            pltpu.VMEM((F // C, C), f32),
            pltpu.VMEM((S // C, C), f32),
            pltpu.VMEM((PR, C), jnp.int32),
            pltpu.SemaphoreType.DMA((XD,)),
            pltpu.SemaphoreType.DMA((3, N1)),
            pltpu.SemaphoreType.DMA((N1,)),
            pltpu.SemaphoreType.DMA((N2,)),
            pltpu.SemaphoreType.DMA((S // OC,)),
        ],
        compiler_params=pltpu.CompilerParams(vmem_limit_bytes=110 * 1024 * 1024),
    )(
        A_q.reshape(S, D).T, A_k.reshape(S, D).T, A_v.reshape(S, D).T, A_ssm_k, B_w1, B_w2,
        A_shift_k.T, A_ssm_D, B_b1.reshape(F // C, C), B_b2.reshape(S // C, C),
        jnp.asarray(fw, bf16), jnp.asarray(iv, bf16),
    )
    return out.T.reshape(1, S, D)
```

```python
import jax
import jax.numpy as jnp
import numpy as np
from jax import lax
import jax.experimental.pallas as pl
import jax.experimental.pallas.tpu as pltpu

S, D, F, KS = 2048, 576, 4608, 4
C = 128
NB = S // C
FC = 512
N1 = F // FC
RG = D // N1
SC = 512
N2 = S // SC
OC = 128
TC = 256
NX = S // TC
XD = 4
KC = S // 8
PR = 8
IB = 2
EPS = 1e-5

f32 = jnp.float32
bf16 = jnp.bfloat16


def _dft_mats():
    t = np.arange(C, dtype=np.float64)
    th = 2.0 * np.pi * (np.arange(C, dtype=np.float64) + 0.5) / (2 * C)
    fw = np.concatenate([np.cos(np.outer(t, th)), -np.sin(np.outer(t, th))], axis=1)
    iv = np.concatenate([np.cos(np.outer(th, t)), -np.sin(np.outer(th, t))], axis=0) / C
    return fw.astype(np.float32).astype(bf16), iv.astype(np.float32).astype(bf16)


def _gelu(x):
    c = 0.7978845608028654
    hx = 0.5 * x
    return hx + hx * jnp.tanh(x * (c + (c * 0.044715) * (x * x)))


def _kernel(x_hbm, k_hbm, v_hbm, sk_hbm, w1_hbm, w2_hbm,
            shift_ref, d_ref, b1_ref, b2_ref, fw_ref, iv_ref,
            o_hbm,
            xbuf, kbuf, vbuf, skbuf, w1buf, w2buf, obuf,
            hT, xnT, kvs, ubuf, sT, xf, kf, pk, px, zb, dcol, wsh, b1s, b2s, zmask,
            sem_x, sem_g, sem_w1, sem_w2, sem_o):
    def al(i, n):
        return pl.ds(i * n if isinstance(i, int) else pl.multiple_of(i * n, n), n)

    def x_copy(i):
        return pltpu.make_async_copy(x_hbm.at[:, al(i, S // XD)], xbuf.at[:, al(i, S // XD)],
                                     sem_x.at[i])

    def g_copies(g):
        return [pltpu.make_async_copy(src.at[al(g, RG), :], dst.at[al(g, RG), :], sem_g.at[n, g])
                for n, (src, dst) in enumerate(((k_hbm, kbuf), (v_hbm, vbuf), (sk_hbm, skbuf)))]

    def w1_copy(c):
        return pltpu.make_async_copy(w1_hbm.at[:, al(c, FC)], w1buf.at[c], sem_w1.at[c])

    def w2_copy(p):
        return pltpu.make_async_copy(w2_hbm.at[:, al(p, SC)], w2buf.at[p], sem_w2.at[p])

    def o_copy(h):
        return pltpu.make_async_copy(obuf.at[:, al(h, OC)], o_hbm.at[:, al(h, OC)], sem_o.at[h])

    for i in range(XD):
        x_copy(i).start()
    for cp in g_copies(0) + g_copies(1):
        cp.start()
    w1_copy(0).start()

    dcol[...] = jnp.broadcast_to(d_ref[...].astype(f32).reshape(1, D), (C, D)).T
    sh = shift_ref[...].astype(f32)
    for j in range(KS):
        wsh[j] = jnp.broadcast_to(sh[j:j + 1, :], (C, D)).T
    b1s[...] = b1_ref[...].astype(f32)
    b2s[...] = b2_ref[...].astype(f32)
    zb[...] = jnp.zeros(zb.shape, bf16)
    zmask[...] = jnp.zeros(zmask.shape, jnp.int32)

    def ln_body(i, _):
        @pl.when(i % (NX // XD) == 0)
        def _():
            x_copy(i // (NX // XD)).wait()

        xt = xbuf[:, al(i, TC)].astype(f32)
        m = jnp.sum(xt, axis=0, keepdims=True) * (1.0 / D)
        xc = xt - m
        v = jnp.sum(xc * xc, axis=0, keepdims=True) * (1.0 / D)
        r = lax.rsqrt(v + EPS)
        xn = xc * r
        r2 = lax.rsqrt(v * (r * r) + EPS)
        xnT[:, al(i, TC)] = xn.astype(bf16)
        hT[:, al(i, TC)] = (xn * r2).astype(bf16)
        return 0

    lax.fori_loop(0, NX, ln_body, 0)

    lane = lax.broadcasted_iota(jnp.int32, (16, C), 1)
    sgn = 1.0 - 2.0 * (lax.broadcasted_iota(jnp.int32, (PR, C), 1) & 1).astype(f32)

    def kv_stage(g):
        r0 = g * RG if isinstance(g, int) else pl.multiple_of(g * RG, RG)
        for sb in range(RG // 16):
            rows = pl.ds(r0 + sb * 16, 16)
            w = [wsh[j, rows, :] for j in range(KS)]
            prev = None
            for t in range(NB):
                kc = kbuf[rows, t * C:(t + 1) * C].astype(f32)
                rolled = [pltpu.roll(kc, j, axis=1) for j in range(1, KS)]
                acc = kc * w[0]
                for j in range(1, KS):
                    if prev is None:
                        shifted = jnp.where(lane < j, 0.0, rolled[j - 1])
                    else:
                        shifted = jnp.where(lane < j, prev[j - 1], rolled[j - 1])
                    acc = acc + shifted * w[j]
                prev = rolled
                kv = acc * vbuf[rows, t * C:(t + 1) * C].astype(f32)
                kvs[t * RG + sb * 16:t * RG + (sb + 1) * 16, :] = kv.astype(bf16)

    def dft_stage(g):
        r0 = g * RG if isinstance(g, int) else pl.multiple_of(g * RG, RG)
        xf[...] = jnp.dot(kvs[...], fw_ref[...], preferred_element_type=f32)
        lk = jnp.concatenate(
            [skbuf[pl.ds(r0, RG), m * C:(m + 1) * C] for m in range(NB)], axis=0)
        kf[...] = jnp.dot(lk, fw_ref[...], preferred_element_type=f32)

    def idft_stage(g):
        r0 = g * RG if isinstance(g, int) else pl.multiple_of(g * RG, RG)
        y = jnp.dot(zb[...], iv_ref[...], preferred_element_type=f32)
        for i in range(NB):
            q = xnT[pl.ds(r0, RG), i * C:(i + 1) * C].astype(f32)
            sT[pl.ds(r0, RG), i * C:(i + 1) * C] = (q * y[i * RG:(i + 1) * RG, :]).astype(bf16)

    def mac_stage(g):
        r0 = g * RG if isinstance(g, int) else pl.multiple_of(g * RG, RG)
        zero = zmask[...]

        def after(val, prev):
            bits = pltpu.bitcast(val, jnp.int32) | (pltpu.bitcast(prev, jnp.int32) & zero)
            return pltpu.bitcast(bits, f32)

        link = None
        for pr in range(RG // PR):
            def ld(ref, j, half, pr=pr):
                return ref[j * RG + pr * PR:j * RG + (pr + 1) * PR, half * C:(half + 1) * C]
            dd = dcol[pl.ds(r0 + pr * PR, PR), :]
            kr_prev = ki_prev = None
            for m in range(NB):
                kr, ki = ld(kf, m, 0), ld(kf, m, 1)
                if m == 0:
                    kr = kr + dd
                    cc, dm = kr, ki
                else:
                    cc = kr - sgn * ki_prev
                    dm = ki + sgn * kr_prev
                kr_prev, ki_prev = kr, ki
                pk[0, m] = cc
                pk[1, m] = dm - cc
                pk[2, m] = cc + dm
            for j in range(NB):
                px[j] = ld(xf, j, 0) + ld(xf, j, 1)
            for i0 in range(0, NB, IB):
                acc = [[None] * 3 for _ in range(IB)]
                kc = {}
                for j in range(i0 + IB):
                    a, b_, ab = ld(xf, j, 0), ld(xf, j, 1), px[j]
                    for t in range(IB):
                        m = i0 + t - j
                        if m < 0:
                            continue
                        if m not in kc:
                            kc[m] = (pk[0, m], pk[1, m], pk[2, m])
                        k0, k1, k2 = kc[m]
                        ps = (k0 * ab, a * k1, b_ * k2)
                        for q in range(3):
                            if acc[t][q] is not None:
                                acc[t][q] = acc[t][q] + ps[q]
                            elif link is None:
                                acc[t][q] = ps[q]
                            else:
                                acc[t][q] = after(ps[q], link[t][q])
                    kc = {m: val for m, val in kc.items() if m >= i0 - j}
                link = acc
                for t in range(IB):
                    s1, s2, s3 = acc[t]
                    rows = slice((i0 + t) * RG + pr * PR, (i0 + t) * RG + (pr + 1) * PR)
                    zb[rows, 0:C] = (s1 - s3).astype(bf16)
                    zb[rows, C:2 * C] = (s1 + s2).astype(bf16)

    for cp in g_copies(0):
        cp.wait()
    kv_stage(0)
    dft_stage(0)

    def p1_body(c, _):
        w1_copy(c).wait()

        @pl.when(c + 1 < N1)
        def _():
            for cp in g_copies(c + 1):
                cp.wait()
            w1_copy(c + 1).start()

        @pl.when(c + 2 < N1)
        def _():
            for cp in g_copies(c + 2):
                cp.start()

        @pl.when(c + 2 >= N1)
        def _():
            w2_copy(c + 2 - N1).start()

        idft_stage(jnp.maximum(c - 1, 0))
        mac_stage(c)
        gn = jnp.minimum(c + 1, N1 - 1)
        kv_stage(gn)
        dft_stage(gn)
        u = jnp.dot(hT[:, 0:KC], w1buf[c, 0:KC, :], preferred_element_type=f32)
        for kk in range(1, S // KC):
            u = u + jnp.dot(hT[:, kk * KC:(kk + 1) * KC], w1buf[c, kk * KC:(kk + 1) * KC, :],
                            preferred_element_type=f32)
        for t in range(FC // C):
            cols = slice(t * C, (t + 1) * C)
            ut = u[:, cols] + b1s[pl.ds(c * (FC // C) + t, 1), :]
            ubuf[c, :, cols] = _gelu(ut).astype(bf16)
        return 0

    lax.fori_loop(0, N1, p1_body, 0, unroll=3)
    idft_stage(N1 - 1)

    def p2_body(p, _):
        @pl.when(p + 2 < N2)
        def _():
            w2_copy(p + 2).start()

        w2_copy(p).wait()
        acc = jnp.dot(ubuf[0], w2buf[p, 0:FC, :], preferred_element_type=f32)
        for c in range(1, N1):
            acc = acc + jnp.dot(ubuf[c], w2buf[p, c * FC:(c + 1) * FC, :],
                                preferred_element_type=f32)
        for h in range(SC // OC):
            oc = p * (SC // OC) + h
            nt = OC // C
            b2c = b2s[pl.ds(oc * nt, nt), :]
            y = acc[:, h * OC:(h + 1) * OC] + jnp.concatenate(
                [b2c[t:t + 1, :] for t in range(nt)], axis=1)
            g = y * jax.nn.sigmoid(y)
            obuf[:, al(oc, OC)] = (
                xbuf[:, al(oc, OC)].astype(f32) + sT[:, al(oc, OC)].astype(f32) * g).astype(bf16)
            o_copy(oc).start()
        return 0

    lax.fori_loop(0, N2, p2_body, 0)
    for h in range(S // OC):
        o_copy(h).wait()


@jax.jit
def pallas_recurrent_scan__ssm_conv_h3__mixer_token_mlp__prompt_kernel(
    A_q: jax.Array,
    A_k: jax.Array,
    A_v: jax.Array,
    A_shift_k: jax.Array,
    A_ssm_k: jax.Array,
    A_ssm_D: jax.Array,
    B_x: jax.Array,
    B_w1: jax.Array,
    B_b1: jax.Array,
    B_w2: jax.Array,
    B_b2: jax.Array,
):
    del B_x
    fw, iv = _dft_mats()
    hbm_spec = pl.BlockSpec(memory_space=pltpu.HBM)
    vmem_spec = pl.BlockSpec(memory_space=pltpu.VMEM)
    out = pl.pallas_call(
        _kernel,
        out_shape=jax.ShapeDtypeStruct((D, S), bf16),
        in_specs=[hbm_spec] * 6 + [vmem_spec] * 6,
        out_specs=hbm_spec,
        scratch_shapes=[
            pltpu.VMEM((D, S), bf16),
            pltpu.VMEM((D, S), bf16),
            pltpu.VMEM((D, S), bf16),
            pltpu.VMEM((D, S), bf16),
            pltpu.VMEM((N1, S, FC), bf16),
            pltpu.VMEM((N2, F, SC), bf16),
            pltpu.VMEM((D, S), bf16),
            pltpu.VMEM((D, S), bf16),
            pltpu.VMEM((D, S), bf16),
            pltpu.VMEM((NB * RG, C), bf16),
            pltpu.VMEM((N1, D, FC), bf16),
            pltpu.VMEM((D, S), bf16),
            pltpu.VMEM((NB * RG, 2 * C), f32),
            pltpu.VMEM((NB * RG, 2 * C), f32),
            pltpu.VMEM((3, NB, PR, C), f32),
            pltpu.VMEM((NB, PR, C), f32),
            pltpu.VMEM((NB * RG, 2 * C), bf16),
            pltpu.VMEM((D, C), f32),
            pltpu.VMEM((KS, D, C), f32),
            pltpu.VMEM((F // C, C), f32),
            pltpu.VMEM((S // C, C), f32),
            pltpu.VMEM((PR, C), jnp.int32),
            pltpu.SemaphoreType.DMA((XD,)),
            pltpu.SemaphoreType.DMA((3, N1)),
            pltpu.SemaphoreType.DMA((N1,)),
            pltpu.SemaphoreType.DMA((N2,)),
            pltpu.SemaphoreType.DMA((S // OC,)),
        ],
        compiler_params=pltpu.CompilerParams(vmem_limit_bytes=100 * 1024 * 1024),
    )(
        A_q.reshape(S, D).T, A_k.reshape(S, D).T, A_v.reshape(S, D).T, A_ssm_k, B_w1, B_w2,
        A_shift_k.T, A_ssm_D, B_b1.reshape(F // C, C), B_b2.reshape(S // C, C),
        fw, iv,
    )
    return out.T.reshape(1, S, D)
```
